```python
import jax
import jax.numpy as jnp

def _softmax(x, axis=-1):
    return jax.nn.softmax(x, axis=axis)

def _gelu(x):
    return jax.nn.gelu(x, approximate=True)

def _silu(x):
    return jax.nn.silu(x)

def _sigmoid(x):
    return jax.nn.sigmoid(x)

def _layernorm(x, axis=-1, eps=1e-05):
    m = jnp.mean(x, axis=axis, keepdims=True)
    v = jnp.var(x, axis=axis, keepdims=True)
    return (x - m) / jnp.sqrt(v + eps)

def _scatter_add(tgt, idx, src, axis=0):
    return tgt.at[idx].add(src)

def _segment_sum(src, seg, n):
    return jax.ops.segment_sum(src, seg, n)

class _Rng:

    def __init__(self, key):
        self._k = key

    def _next(self):
        self._k, sub = jax.random.split(self._k)
        return sub

    def normal(self, shape):
        return jax.random.normal(self._next(), shape, dtype=jnp.bfloat16)

    def randint(self, lo, hi, shape):
        return jax.random.randint(self._next(), shape, lo, hi, dtype=jnp.int32)

    def uniform(self, shape, lo=0.0, hi=1.0):
        return jax.random.uniform(self._next(), shape, jnp.bfloat16, lo, hi)

    def permutation(self, n):
        return jax.random.permutation(self._next(), n)
kernel_name = 'adaLN_cond__memory_aug_infini_attn__dense_activation_gelu__prompt'

def _fwd_setup_inputs():
    _rng = _Rng(jax.random.key(int.from_bytes(__import__("os").urandom(4), "little")))
    _w = lambda a: (lambda t: t.astype(jnp.bfloat16) if jnp.issubdtype(t.dtype, jnp.floating) else t)(jnp.asarray(a))

    def _A_setup():
        B, S, D, H = (1, 2048, 640, 32)
        N = 4
        L = max(1, S // N)
        sc = D ** (-0.5)
        return {'x': _w((lambda *s: _rng.normal(s) * 0.05)(B, N * L, D)), 'wq': _w((lambda *s: _rng.normal(s) * 0.05)(D, D) * sc), 'wk': _w((lambda *s: _rng.normal(s) * 0.05)(D, D) * sc), 'wv': _w((lambda *s: _rng.normal(s) * 0.05)(D, D) * sc), 'wo': _w((lambda *s: _rng.normal(s) * 0.05)(D, D) * sc), 'beta': _w((lambda *s: _rng.normal(s) * 0.05)(H))}
    _A_in = _A_setup()

    def _B_setup():
        B, S, D, F = (1, 2048, 640, 1728)
        return {'x': _w((lambda *s: _rng.normal(s) * 0.05)(B, S, D)), 'w1': _w((lambda *s: _rng.normal(s) * 0.05)(D, F) * D ** (-0.5)), 'b1': _w((lambda *s: _rng.normal(s) * 0.05)(F) * 0.01), 'w2': _w((lambda *s: _rng.normal(s) * 0.05)(F, D) * F ** (-0.5)), 'b2': _w((lambda *s: _rng.normal(s) * 0.05)(D) * 0.01)}
    _B_in = _B_setup()
    return {'A_x': _A_in['x'], 'A_wq': _A_in['wq'], 'A_wk': _A_in['wk'], 'A_wv': _A_in['wv'], 'A_wo': _A_in['wo'], 'A_beta': _A_in['beta'], 'B_x': _B_in['x'], 'B_w1': _B_in['w1'], 'B_b1': _B_in['b1'], 'B_w2': _B_in['w2'], 'B_b2': _B_in['b2'], 'c': _w((lambda *s: _rng.normal(s) * 0.05)(1, 640)), 'w_mod': _w((lambda *s: _rng.normal(s) * 0.05)(640, 6 * 640) * 640 ** (-0.5))}

def _fwd_reference(A_x, A_wq, A_wk, A_wv, A_wo, A_beta, B_x, B_w1, B_b1, B_w2, B_b2, c, w_mod):

    def _A_ref(x, wq, wk, wv, wo, beta):
        B, S, D = x.shape
        H = 32
        Dh = D // H
        N = 4
        L = S // N
        q = (lambda x, *d: x.transpose(*d))((x @ wq).reshape(B, S, H, Dh), 0, 2, 1, 3).reshape(B, H, N, L, Dh)
        k = (lambda x, *d: x.transpose(*d))((x @ wk).reshape(B, S, H, Dh), 0, 2, 1, 3).reshape(B, H, N, L, Dh)
        v = (lambda x, *d: x.transpose(*d))((x @ wv).reshape(B, S, H, Dh), 0, 2, 1, 3).reshape(B, H, N, L, Dh)
        phi = lambda t: jnp.where(t > 0, t + 1.0, jnp.exp(t))
        scale = Dh ** (-0.5)
        ar = jnp.arange(L)
        mask = (lambda x, dt: x.astype(dt))(ar[:, None] < ar[None, :], x.dtype) * -1000000000.0
        g = _sigmoid(beta).reshape(1, H, 1, 1)
        M = jnp.einsum('bhd,bhe->bhde', q[:, :, 0, 0, :] * 0.0, q[:, :, 0, 0, :] * 0.0)
        z = q[:, :, 0, 0, :] * 0.0
        outs = []
        for s in range(N):
            qs, ks, vs = (q[:, :, s].copy(), k[:, :, s].copy(), v[:, :, s].copy())
            logits = jnp.einsum('bhqd,bhkd->bhqk', qs, ks) * scale + mask
            p = _softmax(logits, axis=-1)
            a_dot = jnp.einsum('bhqk,bhkd->bhqd', p, vs)
            pq = phi(qs)
            num = jnp.einsum('bhld,bhde->bhle', pq, M)
            den = jnp.einsum('bhld,bhd->bhl', pq, z)[..., None] + 1e-06
            a_mem = num / den
            o = g * a_mem + (1.0 - g) * a_dot
            outs.append(o)
            pk = phi(ks)
            M = M + jnp.einsum('bhld,bhle->bhde', pk, vs)
            z = z + jnp.einsum('bhld->bhd', pk)
        o = (lambda x, *d: x.transpose(*d))(jnp.stack(outs, 2).reshape(B, H, S, Dh), 0, 2, 1, 3).reshape(B, S, D)
        return o @ wo

    def _B_ref(x, w1, b1, w2, b2):
        h = jnp.einsum('bsd,df->bsf', x, w1) + b1
        h = _gelu(h)
        return jnp.einsum('bsf,fd->bsd', h, w2) + b2
    x = A_x
    mod = (_silu(c) @ w_mod).reshape(c.shape[0], 6, 1, -1)
    sa, ca, ga, sb, cb, gb = (mod[:, 0].copy(), mod[:, 1].copy(), mod[:, 2].copy(), mod[:, 3].copy(), mod[:, 4].copy(), mod[:, 5].copy())
    h = _layernorm(x, axis=-1) * (1 + ca) + sa
    x = x + ga * _A_ref(h, A_wq, A_wk, A_wv, A_wo, A_beta)
    h = _layernorm(x, axis=-1) * (1 + cb) + sb
    x = x + gb * _B_ref(h, B_w1, B_b1, B_w2, B_b2)
    return x

def setup_inputs():
    _inp = _fwd_setup_inputs()
    _gk = jax.random.fold_in(jax.random.key(int.from_bytes(__import__("os").urandom(4), "little")), 2 ** 31 - 1)
    _shapes = [[1, 2048, 640]]
    _dtypes = ['bfloat16']
    _gks = jax.random.split(_gk, len(_shapes))
    _gs = [jax.random.normal(k, s, dtype=jnp.dtype(d)) * 0.05 for k, s, d in zip(_gks, _shapes, _dtypes)]
    _inp['grad_out'] = _gs[0]
    return _inp

def reference(A_x, A_wq, A_wk, A_wv, A_wo, A_beta, B_w1, B_b1, B_w2, B_b2, c, w_mod, B_x, grad_out):
    _const = dict(B_x=B_x)

    def _f(*_d):
        return _fwd_reference(**{'A_x': _d[0], 'A_wq': _d[1], 'A_wk': _d[2], 'A_wv': _d[3], 'A_wo': _d[4], 'A_beta': _d[5], 'B_w1': _d[6], 'B_b1': _d[7], 'B_w2': _d[8], 'B_b2': _d[9], 'c': _d[10], 'w_mod': _d[11], **_const})
    _out, _vjp = jax.vjp(_f, A_x, A_wq, A_wk, A_wv, A_wo, A_beta, B_w1, B_b1, B_w2, B_b2, c, w_mod)
    _grads = _vjp(grad_out)
    _out0 = jnp.asarray(_out)
    return (_out0, *[jnp.asarray(_g) for _g in _grads])
```

```python
import math

import jax
import jax.numpy as jnp
from jax import lax
import jax.experimental.pallas as pl
import jax.experimental.pallas.tpu as pltpu

S, D, H, DH, NSEG, L, F = 2048, 640, 32, 20, 4, 512, 1728
GR = 80
NG = D // GR
NT = L // 128
EROWS = 128 * NT * (NT + 1) // 2
EOFF = [128 * t * (t + 1) // 2 for t in range(NT)]
SCALE = DH ** (-0.5)
LOG2E = math.log2(math.e)
LN_EPS = 1e-5
DEN_EPS = 1e-6
NEG = -1e30
FCHUNKS = [(0, 512), (512, 512), (1024, 512), (1536, 192)]

f32 = jnp.float32
bf16 = jnp.bfloat16

_NN = (((1,), (0,)), ((), ()))
_NT = (((1,), (1,)), ((), ()))
_TN = (((0,), (0,)), ((), ()))
_TT = (((0,), (1,)), ((), ()))


def _dot(a, b, dn):
    return lax.dot_general(a, b, dn, preferred_element_type=f32)


def _phi(t):
    return jnp.where(t > 0, t + 1.0, jnp.exp(t))


def _rows(shape):
    return lax.broadcasted_iota(jnp.int32, shape, 0)


def _cols(shape):
    return lax.broadcasted_iota(jnp.int32, shape, 1)


def _merge(parts):
    n = parts[0].shape[1]
    lo = _rows((8, n)) < 4
    a0, a1, a2, a3 = parts
    return jnp.concatenate([
        a0[0:16], jnp.where(lo, a0[16:24], a1[0:8]), a1[8:24],
        a2[0:16], jnp.where(lo, a2[16:24], a3[0:8]), a3[8:24]], axis=0)


def _expand(tiles):
    n = tiles[0].shape[1]
    lo = _rows((8, n)) < 4
    t0, t1, t2, t3 = tiles
    return jnp.concatenate([
        t0, t0, jnp.where(lo, t0, t1), t1, t1,
        t2, t2, jnp.where(lo, t2, t3), t3, t3], axis=0)


def _head_sums(a):
    n = a.shape[1]
    lo = _rows((8, n)) < 4
    z = jnp.zeros((8, n), a.dtype)
    p = [
        a[0:8] + a[8:16] + jnp.where(lo, a[16:24], z),
        jnp.where(lo, z, a[16:24]) + a[24:32] + a[32:40],
        a[40:48] + a[48:56] + jnp.where(lo, a[56:64], z),
        jnp.where(lo, z, a[56:64]) + a[64:72] + a[72:80],
    ]
    return [jnp.sum(t, axis=0, keepdims=True) for t in p]


def _lane_fold(a):
    return (a[:, 0:128] + a[:, 128:256]) + (a[:, 256:384] + a[:, 384:512])


def _ln_stats(x):
    mu = jnp.mean(x, axis=-1, keepdims=True)
    xc = x - mu
    var = jnp.mean(xc * xc, axis=-1, keepdims=True)
    rstd = lax.rsqrt(var + LN_EPS)
    return xc * rstd, rstd


def _ln_bwd(dxhat, xhat, rstd):
    m1 = jnp.mean(dxhat, axis=-1, keepdims=True)
    m2 = jnp.mean(dxhat * xhat, axis=-1, keepdims=True)
    return rstd * (dxhat - m1 - xhat * m2)


def _colsum8(a):
    r, n = a.shape
    return jnp.sum(a.reshape(r // 8, 8, n), axis=0)


def _kernel(x_hbm, g_hbm, wq_hbm, wk_hbm, wv_hbm, wo_hbm, w1_hbm, w2_hbm, wmod_hbm,
            beta_ref, b1_ref, b2_ref, c_ref,
            out_hbm, dx_hbm, dwq_hbm, dwk_hbm, dwv_hbm, dwo_hbm, dw1_hbm, dw2_hbm, dwmod_hbm,
            dbeta_ref, db1_ref, db2_ref, dc_ref,
            x_ref, g_ref, wqkv_ref, wo_ref, w1_ref, w2_ref, wmod_ref,
            out_v, dx_v, dwqkv_v, dwo_v, dw1_v, dw2_v, dwmod_v,
            mod_s, gate_s, h1_s, qkv_s, ktm_s, vtm_s, mt_s, dmt_s, e_s, st0, st1, m0, m1,
            linv_s, dinv_s, adot_s, amem_s, ot_s, dot_s, dqkv_s, dx1_s,
            awqkv_s, awo_s, aw1_s, aw2_s, avec_s, ab1_s, adg_s, dsc_s,
            isem, osem):
    st_s = (st0, st1)
    m_s = (m0, m1)

    def cp(src, dst, sem):
        return pltpu.make_async_copy(src, dst, sem)

    in_wmod0 = cp(wmod_hbm.at[:, 0:2 * D], wmod_ref.at[:, 0:2 * D], isem.at[0])
    in_x0 = cp(x_hbm.at[0:L], x_ref.at[0:L], isem.at[1])
    in_wq = cp(wq_hbm, wqkv_ref.at[0], isem.at[2])
    in_wk = cp(wk_hbm, wqkv_ref.at[1], isem.at[3])
    in_wv = cp(wv_hbm, wqkv_ref.at[2], isem.at[4])
    in_x1 = cp(x_hbm.at[L:S], x_ref.at[L:S], isem.at[5])
    in_wmod1 = cp(wmod_hbm.at[:, 2 * D:6 * D], wmod_ref.at[:, 2 * D:6 * D], isem.at[6])
    in_wo = cp(wo_hbm, wo_ref, isem.at[7])
    in_w1 = cp(w1_hbm, w1_ref, isem.at[8])
    in_w2 = cp(w2_hbm, w2_ref, isem.at[9])
    in_g = cp(g_hbm, g_ref, isem.at[10])

    def out_seg(s):
        r0 = pl.multiple_of(s * L, L)
        return cp(out_v.at[pl.ds(r0, L)], out_hbm.at[pl.ds(r0, L)], osem.at[s])

    def dx_seg(s):
        r0 = pl.multiple_of(s * L, L)
        return cp(dx_v.at[pl.ds(r0, L)], dx_hbm.at[pl.ds(r0, L)], osem.at[NSEG + s])

    o_dwqkv = [cp(dwqkv_v.at[i], dst, osem.at[8 + i])
               for i, dst in enumerate((dwq_hbm, dwk_hbm, dwv_hbm))]
    o_dwo = cp(dwo_v, dwo_hbm, osem.at[11])
    o_dw1 = cp(dw1_v, dw1_hbm, osem.at[12])
    o_dw2 = cp(dw2_v, dw2_hbm, osem.at[13])
    o_dwmod0 = cp(dwmod_v.at[:, 0:2 * D], dwmod_hbm.at[:, 0:2 * D], osem.at[14])
    o_dwmod1 = cp(dwmod_v.at[:, 2 * D:6 * D], dwmod_hbm.at[:, 2 * D:6 * D], osem.at[15])

    for d in (in_wmod0, in_x0, in_wq, in_wk, in_wv):
        d.start()
    for r in (awqkv_s, awo_s, aw1_s, aw2_s, avec_s, ab1_s, adg_s, dmt_s):
        r[...] = jnp.zeros(r.shape, r.dtype)
    mt_s[0] = jnp.zeros(mt_s.shape[1:], f32)
    c = c_ref[...].astype(f32)
    sig_c = jax.nn.sigmoid(c)
    silu_c = c * sig_c
    silu8 = jnp.broadcast_to(silu_c, (16, D)).astype(bf16)
    gate = jax.nn.sigmoid(beta_ref[...].astype(f32))
    hsel = (_rows((D, H)) // DH) == _cols((D, H))
    gcol = jnp.sum(jnp.where(hsel, gate, 0.0), axis=1, keepdims=True)
    gate_s[...] = jnp.broadcast_to(gcol, (D, 128))
    in_wmod0.wait()
    mod_s[:, 0:2 * D] = _dot(silu8, wmod_ref[:, 0:2 * D], _NN)
    for d in (in_x0, in_wq, in_wk, in_wv):
        d.wait()
    for d in (in_x1, in_wmod1, in_wo, in_w1, in_w2, in_g):
        d.start()

    def modv(i):
        return mod_s[0:1, i * D:(i + 1) * D]

    mr = _rows((96, GR))
    mc = _cols((96, GR)) // DH
    mem_mask = jnp.where(mr < GR, mr // DH, mr - GR) == mc

    def phase1(s, carry):
        @pl.when(s == 1)
        def _():
            in_x1.wait()

        r0 = pl.multiple_of(s * L, L)
        x = x_ref[pl.ds(r0, L), :].astype(f32)
        xhat, _ = _ln_stats(x)
        h1 = (xhat * (1.0 + modv(1)) + modv(0)).astype(bf16)
        h1_s[s] = h1
        kt = _dot(wqkv_ref[1], h1, _TT)
        vt = _dot(wqkv_ref[2], h1, _TT)
        qt = _dot(wqkv_ref[0], h1, _TT)
        qkv_s[s, 0] = qt.astype(bf16)
        qkv_s[s, 3] = (qt * (SCALE * LOG2E)).astype(bf16)
        qkv_s[s, 1] = kt.astype(bf16)
        qkv_s[s, 2] = vt.astype(bf16)
        ones = jnp.ones((16, L), bf16)
        for g in range(NG):
            rs = slice(g * GR, (g + 1) * GR)
            ktm_s[s, g] = jnp.concatenate(
                [kt[rs], jnp.zeros((48, L), f32)], axis=0).T.astype(bf16)
            vtm_s[s, g] = jnp.concatenate(
                [vt[rs], jnp.ones((16, L), f32), jnp.zeros((32, L), f32)], axis=0).T.astype(bf16)
        for g in range(NG):
            rs = slice(g * GR, (g + 1) * GR)
            mt = mt_s[s, g]
            pk = _phi(qkv_s[s, 1, rs, :].astype(f32)).astype(bf16)
            vx = jnp.concatenate([qkv_s[s, 2, rs, :], ones], axis=0)
            upd = _dot(vx, pk, _NT)
            mt_s[s + 1, g] = mt + jnp.where(mem_mask, upd, 0.0)
            pq = _phi(qkv_s[s, 0, rs, :].astype(f32)).astype(bf16)
            numx = _dot(mt.astype(bf16), pq, _NN)
            dinvs = [jnp.broadcast_to(1.0 / (numx[GR + j:GR + j + 1] + DEN_EPS), (8, L))
                     for j in range(4)]
            dinv_s[s, g] = jnp.concatenate(dinvs, axis=0)
            amem_s[s, rs, :] = numx[0:GR] * _expand(dinvs)
        return carry

    with jax.named_scope('phase1'):
        lax.fori_loop(0, NSEG, phase1, 0)

    in_wmod1.wait()
    mod_s[:, 2 * D:6 * D] = _dot(silu8, wmod_ref[:, 2 * D:6 * D], _NN)
    for d in (in_wo, in_w1, in_w2, in_g):
        d.wait()

    causal = _rows((128, 128)) <= _cols((128, 128))
    causal = jnp.concatenate([causal] * 4, axis=1)
    wrow = _rows((32, L))
    r16 = _rows((16, L))
    inh = [(wrow >= 4 * j) & (wrow < 4 * j + DH) for j in range(4)]
    los = (0, 0, 8, 8)

    def mod_grads(lo, hi):
        sc_col = jnp.broadcast_to(silu_c, (128, D)).T
        sc_col = jnp.concatenate([sc_col] * (D // 128), axis=1)
        r = _rows((16, D))
        dsc = jnp.zeros((16, D), f32)
        for i in range(lo, hi):
            dm = jnp.sum(avec_s[i], axis=0, keepdims=True)
            dwmod_v[:, i * D:(i + 1) * D] = (sc_col * dm).astype(bf16)
            hi_p = dm.astype(bf16).astype(f32)
            lhs = jnp.where(r == 0, hi_p, jnp.where(r == 1, dm - hi_p, 0.0)).astype(bf16)
            dsc = dsc + _dot(lhs, wmod_ref[:, i * D:(i + 1) * D], _NT)
        return dsc

    def phase2(i, carry):
        s = NSEG - 1 - i
        r0 = pl.multiple_of(s * L, L)
        last = i == NSEG - 1

        def a_prep(g):
            g0 = pl.multiple_of(g * GR, 16)
            qs = qkv_s[s, 3, pl.ds(g0, GR), :]
            rhs = []
            for j in range(4):
                qw = jnp.where(inh[j], qs[16 * j:16 * j + 32].astype(f32), 0.0).astype(bf16)
                pieces = []
                if j > 0:
                    pieces.append(jnp.zeros((16 * j, L), bf16))
                pieces.append(qw)
                pieces.append(jnp.zeros((96 - 16 * j, L), bf16))
                rhs.append(jnp.concatenate(pieces, axis=0))
            return rhs

        def a_tile(g, rhs, slot, t):
            n = 128 * (t + 1)
            r = jnp.concatenate([rhs[j][:, 128 * t:128 * (t + 1)] for j in range(4)], axis=1)
            st = _dot(ktm_s[s, g, 0:n, :], r, _NN)
            diag = jnp.where(causal, st[n - 128:n], NEG)
            st = jnp.concatenate([st[0:n - 128], diag], axis=0) if t > 0 else diag
            st_s[slot][EOFF[t]:EOFF[t] + n, :] = st
            m_s[slot][t] = jnp.broadcast_to(jnp.max(st, axis=0, keepdims=True), (8, 4 * 128))

        def b_prep(g):
            g0 = pl.multiple_of(g * GR, 16)
            vt = qkv_s[s, 2, pl.ds(g0, GR), :]
            return [jnp.where(inh[j], vt[16 * j:16 * j + 32].astype(f32), 1.0).astype(bf16)
                    for j in range(4)]

        def b_tile(g, vws, slot, t):
            n = 128 * (t + 1)
            e32 = jnp.exp2(st_s[slot][EOFF[t]:EOFF[t] + n, :] - m_s[slot][t][0:1])
            e_s[g, EOFF[t]:EOFF[t] + n, :] = e32.astype(bf16)
            return [_dot(vws[j][:, 0:n], e32[:, 128 * j:128 * (j + 1)].astype(bf16), _NN)
                    for j in range(4)]

        def b_fin(g, pv):
            g0 = pl.multiple_of(g * GR, 16)
            parts, linvs = [], []
            for j in range(4):
                ow = jnp.concatenate([pv[t][j] for t in range(NT)], axis=1)
                linv = 1.0 / (ow[24:32] if j < 2 else ow[0:8])
                linvs.append(linv)
                parts.append(ow[los[j]:los[j] + 24] * jnp.concatenate([linv] * 3, axis=0))
            adot = _merge(parts)
            linv_s[g] = jnp.concatenate(linvs, axis=0)
            adot_s[pl.ds(g0, GR), :] = adot
            gt = jnp.concatenate([gate_s[pl.ds(g0, GR), :]] * NT, axis=1)
            amem = amem_s[s, pl.ds(g0, GR), :]
            ot_s[pl.ds(g0, GR), :] = (gt * amem + (1.0 - gt) * adot).astype(bf16)

        def ab(g, slot):
            rhs = a_prep(g + 1)
            vws = b_prep(g)
            pv = []
            for t in range(NT):
                a_tile(g + 1, rhs, 1 - slot, t)
                pv.append(b_tile(g, vws, slot, t))
            b_fin(g, pv)

        def fwd_pair(p, cc):
            ab(2 * p, 0)
            ab(2 * p + 1, 1)
            return cc

        with jax.named_scope('attn_fwd'):
            rhs0 = a_prep(0)
            for t in range(NT):
                a_tile(0, rhs0, 0, t)
            lax.fori_loop(0, NG // 2 - 1, fwd_pair, 0)
            ab(NG - 2, 0)
            vws = b_prep(NG - 1)
            b_fin(NG - 1, [b_tile(NG - 1, vws, 1, t) for t in range(NT)])

        ot = ot_s[...]
        att = _dot(ot, wo_ref[...], _TN)
        x = x_ref[pl.ds(r0, L), :].astype(f32)
        x1 = x + modv(2) * att
        xhat2, rstd2 = _ln_stats(x1)
        h2 = (xhat2 * (1.0 + modv(4)) + modv(3)).astype(bf16)
        gout = g_ref[pl.ds(r0, L), :].astype(f32)
        dff = gout * modv(5)
        df = dff.astype(bf16)
        facc = jnp.zeros((L, D), f32)
        dh2 = jnp.zeros((L, D), f32)
        k0 = math.sqrt(2.0 / math.pi)
        k1 = 0.044715
        for (c0, cw) in FCHUNKS:
            cs = slice(c0, c0 + cw)
            da = _dot(df, w2_ref[cs, :], _NT)
            u = _dot(h2, w1_ref[cs, :], _NT) + b1_ref[:, cs].astype(f32)
            u2 = u * u
            th = jnp.tanh(u * (k0 + (k0 * k1) * u2))
            hp = 0.5 + 0.5 * th
            a = (u * hp).astype(bf16)
            gp = hp + (0.5 * u) * (1.0 - th * th) * (k0 + (3.0 * k0 * k1) * u2)
            facc = facc + _dot(a, w2_ref[cs, :], _NN)
            duf = da * gp
            du = duf.astype(bf16)
            ab1_s[:, cs] += _colsum8(duf)
            v2 = aw2_s[cs, :] + _dot(a, df, _TN)
            aw2_s[cs, :] = v2
            dw2_v[cs, :] = v2.astype(bf16)
            v1 = aw1_s[cs, :] + _dot(du, h2, _TN)
            aw1_s[cs, :] = v1
            dw1_v[cs, :] = v1.astype(bf16)
            dh2 = dh2 + _dot(du, w1_ref[cs, :], _NN)
        ff = facc + b2_ref[...].astype(f32)
        out_v[pl.ds(r0, L), :] = (x1 + modv(5) * ff).astype(bf16)
        avec_s[5] += _colsum8(gout * ff)
        avec_s[6] += _colsum8(dff)
        avec_s[4] += _colsum8(dh2 * xhat2)
        avec_s[3] += _colsum8(dh2)
        dx1 = gout + _ln_bwd(dh2 * (1.0 + modv(4)), xhat2, rstd2)
        dx1_s[...] = dx1
        avec_s[2] += _colsum8(dx1 * att)
        datt = (dx1 * modv(2)).astype(bf16)
        dot_s[...] = _dot(wo_ref[...], datt, _NT)
        vo = awo_s[...] + _dot(ot, datt, _NN)
        awo_s[...] = vo
        dwo_v[...] = vo.astype(bf16)
        out_seg(s).start()

        @pl.when(last)
        def _():
            o_dw1.start()
            o_dw2.start()
            o_dwo.start()
            dsc_s[...] = mod_grads(2, 6)
            o_dwmod1.start()

        def attn_bwd(g, cc):
            g0 = pl.multiple_of(g * GR, 16)
            do = dot_s[pl.ds(g0, GR), :]
            adot = adot_s[pl.ds(g0, GR), :]
            amem = amem_s[s, pl.ds(g0, GR), :]
            adg_s[pl.ds(g0, GR), :] += _lane_fold(do * (amem - adot))
            gt = jnp.concatenate([gate_s[pl.ds(g0, GR), :]] * NT, axis=1)
            linv = linv_s[g]
            dinv = dinv_s[s, g]
            qt = qkv_s[s, 0, pl.ds(g0, GR), :]
            kt = qkv_s[s, 1, pl.ds(g0, GR), :]
            vt = qkv_s[s, 2, pl.ds(g0, GR), :]
            dop = ((1.0 - gt) * do
                   * _expand([linv[8 * j:8 * j + 8] for j in range(4)])).astype(bf16)
            dopf = dop.astype(f32)
            deltas = _head_sums(dopf * adot)
            rhs = []
            for j in range(4):
                dw = jnp.where(inh[j], dopf[16 * j:16 * j + 32], 0.0).astype(bf16)
                nd = -deltas[j]
                nd_hi = nd.astype(bf16).astype(f32)
                drow = jnp.where(r16 == 0, nd_hi,
                                 jnp.where(r16 == 1, nd - nd_hi, 0.0)).astype(bf16)
                pieces = []
                if j > 0:
                    pieces.append(jnp.zeros((16 * j, L), bf16))
                pieces.append(dw)
                if j < 3:
                    pieces.append(jnp.zeros((48 - 16 * j, L), bf16))
                pieces.append(drow)
                pieces.append(jnp.zeros((32, L), bf16))
                rhs.append(jnp.concatenate(pieces, axis=0))
            kw = [kt[16 * j:16 * j + 32] for j in range(4)]
            qw = [qt[16 * j:16 * j + 32] for j in range(4)]
            dow = [dop[16 * j:16 * j + 32] for j in range(4)]
            dq_t = [[None] * NT for _ in range(4)]
            dk_t = [[None] * NT for _ in range(4)]
            dv_t = [[None] * NT for _ in range(4)]

            def acc(lst, val, t):
                for u in range(t + 1):
                    a = val[:, 128 * u:128 * (u + 1)]
                    lst[u] = a if lst[u] is None else lst[u] + a

            def f_dp(t):
                n = 128 * (t + 1)
                r = jnp.concatenate([rhs[j][:, 128 * t:128 * (t + 1)] for j in range(4)], axis=1)
                dp = _dot(vtm_s[s, g, 0:n, :], r, _NN)
                ds = e_s[g, EOFF[t]:EOFF[t] + n, :].astype(f32) * dp
                return [ds[:, 128 * j:128 * (j + 1)].astype(bf16) for j in range(4)]

            def f_dv(t):
                n = 128 * (t + 1)
                for j in range(4):
                    e = e_s[g, EOFF[t]:EOFF[t] + n, 128 * j:128 * (j + 1)]
                    acc(dv_t[j], _dot(dow[j][:, 128 * t:128 * (t + 1)], e, _NT), t)

            def f_dqk(t, ds):
                n = 128 * (t + 1)
                for j in range(4):
                    dq_t[j][t] = _dot(kw[j][:, 0:n], ds[j], _NN)
                for j in range(4):
                    acc(dk_t[j], _dot(qw[j][:, 128 * t:128 * (t + 1)], ds[j], _NT), t)

            qf = qt.astype(f32)
            kf = kt.astype(f32)
            pqf = _phi(qf)
            pkf = _phi(kf)
            dnum = gt * do * _expand([dinv[8 * j:8 * j + 8] for j in range(4)])
            dds = _head_sums(dnum * amem)
            dden = jnp.zeros((16, L), f32)
            for j in range(4):
                dden = jnp.where(r16 == j, -dds[j], dden)
            dnx = jnp.concatenate([dnum, dden], axis=0).astype(bf16)
            dmt = dmt_s[g]
            dmtb = dmt.astype(bf16)

            f_dv(3)
            ds3 = f_dp(3)
            f_dv(2)
            vx = jnp.concatenate([vt, jnp.ones((16, L), bf16)], axis=0)
            dpk = _dot(dmtb, vx, _TN)
            dvm = _dot(dmtb[0:GR], pkf.astype(bf16), _NN)
            dpq = _dot(mt_s[s, g].astype(bf16), dnx, _TN)
            upd = _dot(dnx, pqf.astype(bf16), _NT)
            dmt_s[g] = dmt + jnp.where(mem_mask, upd, 0.0)
            ds2 = f_dp(2)
            f_dqk(3, ds3)
            f_dv(1)
            ds1 = f_dp(1)
            f_dqk(2, ds2)
            f_dv(0)
            ds0 = f_dp(0)
            f_dqk(1, ds1)
            f_dqk(0, ds0)

            def mg(lst):
                return _merge([jnp.concatenate(lst[j], axis=1)[los[j]:los[j] + 24]
                               for j in range(4)])

            dq = mg(dq_t) * SCALE + dpq * jnp.where(qf > 0, 1.0, pqf)
            dk = mg(dk_t) * SCALE + dpk * jnp.where(kf > 0, 1.0, pkf)
            dv = mg(dv_t) + dvm
            dqkv_s[0, pl.ds(g0, GR), :] = dq.astype(bf16)
            dqkv_s[1, pl.ds(g0, GR), :] = dk.astype(bf16)
            dqkv_s[2, pl.ds(g0, GR), :] = dv.astype(bf16)
            return cc

        with jax.named_scope('attn_bwd'):
            lax.fori_loop(0, NG, attn_bwd, 0)

        h1 = h1_s[s]
        dh1 = jnp.zeros((L, D), f32)
        for idx in range(3):
            dh1 = dh1 + _dot(dqkv_s[idx], wqkv_ref[idx], _TT)
        x = x_ref[pl.ds(r0, L), :].astype(f32)
        xhat, rstd = _ln_stats(x)
        avec_s[1] += _colsum8(dh1 * xhat)
        avec_s[0] += _colsum8(dh1)
        dx = dx1_s[...] + _ln_bwd(dh1 * (1.0 + modv(1)), xhat, rstd)
        dx_v[pl.ds(r0, L), :] = dx.astype(bf16)
        for idx in range(3):
            v = awqkv_s[idx] + _dot(h1, dqkv_s[idx], _TT)
            awqkv_s[idx] = v
            dwqkv_v[idx] = v.astype(bf16)
        dx_seg(s).start()
        return carry

    with jax.named_scope('phase2'):
        lax.fori_loop(0, NSEG, phase2, 0)

    for d in o_dwqkv:
        d.start()
    dsc = dsc_s[...] + mod_grads(0, 2)
    o_dwmod0.start()
    db1_ref[...] = jnp.sum(ab1_s[...], axis=0, keepdims=True).astype(bf16)
    db2_ref[...] = jnp.sum(avec_s[6], axis=0, keepdims=True).astype(bf16)
    dgc = jnp.sum(adg_s[...], axis=1, keepdims=True)
    dg = jnp.sum(jnp.where(hsel, dgc, 0.0), axis=0, keepdims=True)
    dbeta_ref[...] = (dg * gate * (1.0 - gate)).astype(bf16)
    dsilu = sig_c * (1.0 + c * (1.0 - sig_c))
    dc_ref[...] = ((dsc[0:1] + dsc[1:2]) * dsilu).astype(bf16)
    for s in range(NSEG):
        out_seg(s).wait()
        dx_seg(s).wait()
    for d in o_dwqkv + [o_dwo, o_dw1, o_dw2, o_dwmod0, o_dwmod1]:
        d.wait()


@jax.jit
def pallas_adaLN_cond__memory_aug_infini_attn__dense_activation_gelu__prompt_kernel(
    A_x: jax.Array,
    A_wq: jax.Array,
    A_wk: jax.Array,
    A_wv: jax.Array,
    A_wo: jax.Array,
    A_beta: jax.Array,
    B_x: jax.Array,
    B_w1: jax.Array,
    B_b1: jax.Array,
    B_w2: jax.Array,
    B_b2: jax.Array,
    c: jax.Array,
    w_mod: jax.Array,
    grad_out: jax.Array,
):
    sd = jax.ShapeDtypeStruct
    out_shape = (
        sd((S, D), bf16), sd((S, D), bf16),
        sd((D, D), bf16), sd((D, D), bf16), sd((D, D), bf16), sd((D, D), bf16),
        sd((F, D), bf16), sd((F, D), bf16), sd((D, 6 * D), bf16),
        sd((1, H), bf16), sd((1, F), bf16), sd((1, D), bf16), sd((1, D), bf16),
    )
    vm = pltpu.VMEM
    scratch = [
        vm((S, D), bf16), vm((S, D), bf16), vm((3, D, D), bf16), vm((D, D), bf16),
        vm((F, D), bf16), vm((F, D), bf16), vm((D, 6 * D), bf16),
        vm((S, D), bf16), vm((S, D), bf16), vm((3, D, D), bf16), vm((D, D), bf16),
        vm((F, D), bf16), vm((F, D), bf16), vm((D, 6 * D), bf16),
        vm((16, 6 * D), f32),
        vm((D, 128), f32),
        vm((NSEG, L, D), bf16),
        vm((NSEG, 4, D, L), bf16),
        vm((NSEG, NG, L, 128), bf16),
        vm((NSEG, NG, L, 128), bf16),
        vm((NSEG + 1, NG, 96, GR), f32),
        vm((NG, 96, GR), f32),
        vm((NG, EROWS, 512), bf16),
        vm((EROWS, 512), f32), vm((EROWS, 512), f32),
        vm((NT, 8, 512), f32), vm((NT, 8, 512), f32),
        vm((NG, 32, L), f32),
        vm((NSEG, NG, 32, L), f32),
        vm((D, L), f32),
        vm((NSEG, D, L), f32),
        vm((D, L), bf16),
        vm((D, L), f32),
        vm((3, D, L), bf16),
        vm((L, D), f32),
        vm((3, D, D), f32), vm((D, D), f32), vm((F, D), f32), vm((F, D), f32),
        vm((7, 8, D), f32), vm((8, F), f32), vm((D, 128), f32), vm((16, D), f32),
        pltpu.SemaphoreType.DMA((11,)), pltpu.SemaphoreType.DMA((16,)),
    ]
    hbm = pl.BlockSpec(memory_space=pl.ANY)
    vmem = pl.BlockSpec(memory_space=pltpu.VMEM)
    outs = pl.pallas_call(
        _kernel,
        out_shape=out_shape,
        in_specs=[hbm] * 9 + [vmem] * 4,
        out_specs=tuple([hbm] * 9 + [vmem] * 4),
        scratch_shapes=scratch,
        compiler_params=pltpu.CompilerParams(vmem_limit_bytes=125 * 1024 * 1024),
    )(A_x.reshape(S, D), grad_out.reshape(S, D), A_wq, A_wk, A_wv, A_wo, B_w1.T, B_w2, w_mod,
      A_beta.reshape(1, H), B_b1.reshape(1, F), B_b2.reshape(1, D), c)
    (out, dx, dwq, dwk, dwv, dwo, dw1t, dw2, dwmod, dbeta, db1, db2, dc) = outs
    return (out.reshape(1, S, D), dx.reshape(1, S, D), dwq, dwk, dwv, dwo,
            dbeta.reshape(H), dw1t.T, db1.reshape(F), dw2, db2.reshape(D), dc, dwmod)
```

```python
import math

import jax
import jax.numpy as jnp
from jax import lax
import jax.experimental.pallas as pl
import jax.experimental.pallas.tpu as pltpu

S, D, H, DH, NSEG, L, F = 2048, 640, 32, 20, 4, 512, 1728
GR = 80
NG = D // GR
NT = L // 128
EROWS = 128 * NT * (NT + 1) // 2
EOFF = [128 * t * (t + 1) // 2 for t in range(NT)]
SCALE = DH ** (-0.5)
LOG2E = math.log2(math.e)
LN_EPS = 1e-5
DEN_EPS = 1e-6
NEG = -1e30
BWD_UNROLL = 4
BWD_LAG = 2
RB = 32
MEM_STEPS = (1, 3, 5, 8)
FCHUNKS = [(0, 512), (512, 512), (1024, 512), (1536, 192)]

f32 = jnp.float32
bf16 = jnp.bfloat16

_NN = (((1,), (0,)), ((), ()))
_NT = (((1,), (1,)), ((), ()))
_TN = (((0,), (0,)), ((), ()))
_TT = (((0,), (1,)), ((), ()))


def _dot(a, b, dn):
    return lax.dot_general(a, b, dn, preferred_element_type=f32)


def _phi(t):
    return jnp.where(t > 0, t + 1.0, jnp.exp(t))


def _rows(shape):
    return lax.broadcasted_iota(jnp.int32, shape, 0)


def _cols(shape):
    return lax.broadcasted_iota(jnp.int32, shape, 1)


def _merge(parts):
    n = parts[0].shape[1]
    lo = _rows((8, n)) < 4
    a0, a1, a2, a3 = parts
    return jnp.concatenate([
        a0[0:16], jnp.where(lo, a0[16:24], a1[0:8]), a1[8:24],
        a2[0:16], jnp.where(lo, a2[16:24], a3[0:8]), a3[8:24]], axis=0)


def _expand(tiles):
    n = tiles[0].shape[1]
    lo = _rows((8, n)) < 4
    t0, t1, t2, t3 = tiles
    return jnp.concatenate([
        t0, t0, jnp.where(lo, t0, t1), t1, t1,
        t2, t2, jnp.where(lo, t2, t3), t3, t3], axis=0)


def _head_sums(a):
    n = a.shape[1]
    lo = _rows((8, n)) < 4
    z = jnp.zeros((8, n), a.dtype)
    p = [
        a[0:8] + a[8:16] + jnp.where(lo, a[16:24], z),
        jnp.where(lo, z, a[16:24]) + a[24:32] + a[32:40],
        a[40:48] + a[48:56] + jnp.where(lo, a[56:64], z),
        jnp.where(lo, z, a[56:64]) + a[64:72] + a[72:80],
    ]
    return [jnp.sum(t, axis=0, keepdims=True) for t in p]


def _lane_fold(a):
    return (a[:, 0:128] + a[:, 128:256]) + (a[:, 256:384] + a[:, 384:512])


def _ln_stats(x):
    mu = jnp.mean(x, axis=-1, keepdims=True)
    xc = x - mu
    var = jnp.mean(xc * xc, axis=-1, keepdims=True)
    rstd = lax.rsqrt(var + LN_EPS)
    return xc * rstd, rstd


def _ln_bwd(dxhat, xhat, rstd):
    m1 = jnp.mean(dxhat, axis=-1, keepdims=True)
    m2 = jnp.mean(dxhat * xhat, axis=-1, keepdims=True)
    return rstd * (dxhat - m1 - xhat * m2)


def _colsum8(a):
    r, n = a.shape
    return jnp.sum(a.reshape(r // 8, 8, n), axis=0)


def _kernel(x_hbm, g_hbm, wq_hbm, wk_hbm, wv_hbm, wo_hbm, w1_hbm, w2_hbm, wmod_hbm,
            beta_ref, b1_ref, b2_ref, c_ref,
            out_hbm, dx_hbm, dwq_hbm, dwk_hbm, dwv_hbm, dwo_hbm, dw1_hbm, dw2_hbm, dwmod_hbm,
            dbeta_ref, db1_ref, db2_ref, dc_ref,
            x_ref, g_ref, wqkv_ref, wo_ref, w1_ref, w2_ref, wmod_ref,
            dwqkv_v, dwo_v, dw1_v, dw2_v, dwmod_v,
            mod_s, gate_s, h1_s, qkv_s, ktm_s, vtm_s, mt_s, dmt_s, e_s, st0, st1, m0, m1,
            linv_s, dinv_s, adot_s, amem_s, ot_s, dot_s, dqkv_s, dx1_s,
            awqkv_s, awo_s, aw1_s, aw2_s, avec_s, ab1_s, adg_s, da_s, df_s, sccol_s, b1_s, b2_s,
            isem, osem):
    out_v = g_ref
    dx_v = x_ref
    st_s = (st0, st1)
    m_s = (m0, m1)

    def cp(src, dst, sem):
        return pltpu.make_async_copy(src, dst, sem)

    in_wmod0 = cp(wmod_hbm.at[:, 0:2 * D], wmod_ref.at[:, 0:2 * D], isem.at[0])
    in_x0 = cp(x_hbm.at[0:L], x_ref.at[0:L], isem.at[1])
    in_wq = cp(wq_hbm, dwqkv_v.at[0], isem.at[2])
    in_wk = cp(wk_hbm, dwqkv_v.at[1], isem.at[3])
    in_wv = cp(wv_hbm, dwqkv_v.at[2], isem.at[4])
    in_x1 = cp(x_hbm.at[L:2 * L], x_ref.at[L:2 * L], isem.at[5])
    in_x2 = cp(x_hbm.at[2 * L:S], x_ref.at[2 * L:S], isem.at[11])
    in_wmod1 = cp(wmod_hbm.at[:, 2 * D:6 * D], wmod_ref.at[:, 2 * D:6 * D], isem.at[6])
    in_wo = cp(wo_hbm, wo_ref, isem.at[7])
    in_w1 = cp(w1_hbm, w1_ref, isem.at[8])
    in_w2 = cp(w2_hbm, w2_ref, isem.at[9])
    in_g = cp(g_hbm, g_ref, isem.at[10])

    def out_seg(s):
        r0 = pl.multiple_of(s * L, L)
        return cp(out_v.at[pl.ds(r0, L)], out_hbm.at[pl.ds(r0, L)], osem.at[s])

    def dx_seg(s):
        r0 = pl.multiple_of(s * L, L)
        return cp(dx_v.at[pl.ds(r0, L)], dx_hbm.at[pl.ds(r0, L)], osem.at[NSEG + s])

    o_dwqkv = [cp(dwqkv_v.at[i], dst, osem.at[8 + i])
               for i, dst in enumerate((dwq_hbm, dwk_hbm, dwv_hbm))]
    o_dwo = cp(dwo_v, dwo_hbm, osem.at[11])
    o_dw1 = cp(dw1_v, dw1_hbm, osem.at[12])
    o_dw2 = cp(dw2_v, dw2_hbm, osem.at[13])
    o_dwmod0 = cp(dwmod_v.at[:, 0:2 * D], dwmod_hbm.at[:, 0:2 * D], osem.at[14])
    o_dwmod1 = cp(dwmod_v.at[:, 2 * D:6 * D], dwmod_hbm.at[:, 2 * D:6 * D], osem.at[15])

    for d in (in_wmod0, in_x0, in_wk, in_wv):
        d.start()
    for r in (awo_s, avec_s, ab1_s, adg_s, dmt_s, awqkv_s, aw1_s, aw2_s):
        r[...] = jnp.zeros(r.shape, r.dtype)
    mt_s[0] = jnp.zeros(mt_s.shape[1:], f32)
    c = c_ref[...].astype(f32)
    sig_c = jax.nn.sigmoid(c)
    silu_c = c * sig_c
    silu8 = jnp.broadcast_to(silu_c, (16, D)).astype(bf16)
    gate = jax.nn.sigmoid(beta_ref[...].astype(f32))
    hsel = (_rows((D, H)) // DH) == _cols((D, H))
    gcol = jnp.sum(jnp.where(hsel, gate, 0.0), axis=1, keepdims=True)
    gate_s[...] = jnp.broadcast_to(gcol, (D, 128))
    sccol_s[...] = jnp.broadcast_to(silu_c, (128, D)).T
    b1_s[...] = b1_ref[...].astype(f32).reshape(1, F)
    b2_s[...] = b2_ref[...].astype(f32).reshape(1, D)
    in_wmod0.wait()
    in_wq.start()
    in_x1.start()
    mod_s[:, 0:2 * D] = _dot(silu8, wmod_ref[:, 0:2 * D], _NN)
    in_x0.wait()

    def modv(i):
        return mod_s[0:1, i * D:(i + 1) * D]

    mr = _rows((96, GR))
    mc = _cols((96, GR)) // DH
    mem_mask = jnp.where(mr < GR, mr // DH, mr - GR) == mc

    def ln1_fwd(s):
        xhat, _ = _ln_stats(x_ref[s * L:(s + 1) * L, :].astype(f32))
        h1_s[s] = (xhat * (1.0 + modv(1)) + modv(0)).T.astype(bf16)

    def proj(idx, s):
        if s == 0:
            w = dwqkv_v[idx]
            wqkv_ref[idx] = w.T
            return _dot(w, h1_s[s], _TN)
        return _dot(wqkv_ref[idx], h1_s[s], _NN)

    def proj_k(s):
        kt = proj(1, s)
        qkv_s[s, 1] = kt.astype(bf16)
        for g in range(NG):
            ktm_s[s, g] = jnp.concatenate(
                [kt[g * GR:(g + 1) * GR] * (SCALE * LOG2E), jnp.zeros((48, L), f32)],
                axis=0).T.astype(bf16)

    def proj_v(s):
        vt = proj(2, s)
        qkv_s[s, 2] = vt.astype(bf16)
        for g in range(NG):
            vtm_s[s, g] = jnp.concatenate(
                [vt[g * GR:(g + 1) * GR], jnp.ones((16, L), f32), jnp.zeros((32, L), f32)],
                axis=0).T.astype(bf16)

    def proj_q(s):
        qt = proj(0, s)
        qkv_s[s, 0] = qt.astype(bf16)

    def mem_upd(s):
        ones = jnp.ones((16, L), bf16)
        for g in range(NG):
            rs = slice(g * GR, (g + 1) * GR)
            pk = _phi(qkv_s[s, 1, rs, :].astype(f32)).astype(bf16)
            vx = jnp.concatenate([qkv_s[s, 2, rs, :], ones], axis=0)
            upd = _dot(vx, pk, _NT)
            mt_s[s + 1, g] = mt_s[s, g] + jnp.where(mem_mask, upd, 0.0)

    def mem_read(s):
        for g in range(NG):
            rs = slice(g * GR, (g + 1) * GR)
            pq = _phi(qkv_s[s, 0, rs, :].astype(f32)).astype(bf16)
            numx = _dot(mt_s[s, g].astype(bf16), pq, _NN)
            dinvs = [jnp.broadcast_to(1.0 / (numx[GR + j:GR + j + 1] + DEN_EPS), (8, L))
                     for j in range(4)]
            dinv_s[s, g] = jnp.concatenate(dinvs, axis=0)
            amem_s[s, rs, :] = numx[0:GR] * _expand(dinvs)

    ln1_fwd(0)
    in_wk.wait()
    with jax.named_scope('phase1'):
        proj_k(0)
        in_wv.wait()
        in_x2.start()
        for s in range(NSEG):
            if s == 1:
                in_x2.wait()
                for d in (in_wmod1, in_g, in_w2, in_wo, in_w1):
                    d.start()
            if s > 0:
                proj_k(s)
                mem_read(s - 1)
            if s + 1 < NSEG:
                proj_v(s)
                if s == 0:
                    in_wq.wait()
                    in_x1.wait()
                ln1_fwd(s + 1)
                proj_q(s)
                mem_upd(s)
            else:
                proj_q(s)
                proj_v(s)
                mem_read(s)

    in_wmod1.wait()
    mod_s[:, 2 * D:6 * D] = _dot(silu8, wmod_ref[:, 2 * D:6 * D], _NN)
    for d in (in_wo, in_w1, in_w2, in_g):
        d.wait()

    causal = _rows((128, 128)) <= _cols((128, 128))
    causal = jnp.concatenate([causal] * 4, axis=1)
    wrow = _rows((32, L))
    r16 = _rows((16, L))
    inh = [(wrow >= 4 * j) & (wrow < 4 * j + DH) for j in range(4)]
    los = (0, 0, 8, 8)

    def dwmod_cols(lo, hi):
        sc_col = jnp.concatenate([sccol_s[...]] * (D // 128), axis=1)
        for i in range(lo, hi):
            dm = jnp.sum(avec_s[i], axis=0, keepdims=True)
            dwmod_v[:, i * D:(i + 1) * D] = (sc_col * dm).astype(bf16)

    def phase2(i, carry):
        s = NSEG - 1 - i
        r0 = pl.multiple_of(s * L, L)
        last = i == NSEG - 1

        def a_prep(g):
            g0 = pl.multiple_of(g * GR, 16)
            qs = qkv_s[s, 0, pl.ds(g0, GR), :]
            rhs = []
            for j in range(4):
                qw = jnp.where(inh[j], qs[16 * j:16 * j + 32].astype(f32), 0.0).astype(bf16)
                pieces = []
                if j > 0:
                    pieces.append(jnp.zeros((16 * j, L), bf16))
                pieces.append(qw)
                pieces.append(jnp.zeros((96 - 16 * j, L), bf16))
                rhs.append(jnp.concatenate(pieces, axis=0))
            return rhs

        def a_tile(g, rhs, slot, t):
            n = 128 * (t + 1)
            r = jnp.concatenate([rhs[j][:, 128 * t:128 * (t + 1)] for j in range(4)], axis=1)
            st = _dot(ktm_s[s, g, 0:n, :], r, _NN)
            diag = jnp.where(causal, st[n - 128:n], NEG)
            st = jnp.concatenate([st[0:n - 128], diag], axis=0) if t > 0 else diag
            st_s[slot][EOFF[t]:EOFF[t] + n, :] = st
            m_s[slot][t] = jnp.broadcast_to(jnp.max(st, axis=0, keepdims=True), (8, 4 * 128))

        def b_prep(g):
            g0 = pl.multiple_of(g * GR, 16)
            vt = qkv_s[s, 2, pl.ds(g0, GR), :]
            return [jnp.where(inh[j], vt[16 * j:16 * j + 32].astype(f32), 1.0).astype(bf16)
                    for j in range(4)]

        def b_tile(g, vws, slot, t):
            n = 128 * (t + 1)
            e32 = jnp.exp2(st_s[slot][EOFF[t]:EOFF[t] + n, :] - m_s[slot][t][0:1])
            e_s[g, EOFF[t]:EOFF[t] + n, :] = e32.astype(bf16)
            return [_dot(vws[j][:, 0:n], e32[:, 128 * j:128 * (j + 1)].astype(bf16), _NN)
                    for j in range(4)]

        def b_fin(g, pv):
            g0 = pl.multiple_of(g * GR, 16)
            parts, linvs = [], []
            for j in range(4):
                ow = jnp.concatenate([pv[t][j] for t in range(NT)], axis=1)
                linv = 1.0 / (ow[24:32] if j < 2 else ow[0:8])
                linvs.append(linv)
                parts.append(ow[los[j]:los[j] + 24] * jnp.concatenate([linv] * 3, axis=0))
            adot = _merge(parts)
            linv_s[g] = jnp.concatenate(linvs, axis=0)
            adot_s[pl.ds(g0, GR), :] = adot
            gt = jnp.concatenate([gate_s[pl.ds(g0, GR), :]] * NT, axis=1)
            amem = amem_s[s, pl.ds(g0, GR), :]
            ot_s[pl.ds(g0, GR), :] = (gt * amem + (1.0 - gt) * adot).astype(bf16)

        def da_slice(k, w):
            c0 = k * 256 if isinstance(k, int) else pl.multiple_of(k * 256, 256)
            da_s[k, :, 0:w] = _dot(df_s[...], w2_ref[pl.ds(c0, w), :], _NT)

        def ab(g, slot):
            rhs = a_prep(g + 1)
            vws = b_prep(g)
            pv = []
            for t in range(NT):
                a_tile(g + 1, rhs, 1 - slot, t)
                if t == 2 and not (isinstance(g, int) and g == NG - 2):
                    da_slice(g, 256)
                pv.append(b_tile(g, vws, slot, t))
            b_fin(g, pv)

        def fwd_pair(p, cc):
            ab(2 * p, 0)
            ab(2 * p + 1, 1)
            return cc

        with jax.named_scope('attn_fwd'):
            rhs0 = a_prep(0)
            for t in range(NT):
                a_tile(0, rhs0, 0, NT - 1 - t)
                rows = pl.ds(pl.multiple_of(r0 + 128 * t, 128), 128)
                dff = g_ref[rows, :].astype(f32) * modv(5)
                df_s[128 * t:128 * (t + 1), :] = dff.astype(bf16)
                avec_s[6] += _colsum8(dff)
            lax.fori_loop(0, NG // 2 - 1, fwd_pair, 0)
            ab(NG - 2, 0)
            vws = b_prep(NG - 1)
            pv = [b_tile(NG - 1, vws, 1, 0)]
            att = _dot(ot_s[0:256, :], wo_ref[0:256, :], _TN)
            pv += [b_tile(NG - 1, vws, 1, t) for t in range(1, 3)]
            att = att + _dot(ot_s[256:512, :], wo_ref[256:512, :], _TN)
            pv.append(b_tile(NG - 1, vws, 1, 3))
            b_fin(NG - 1, pv)

        att = att + _dot(ot_s[512:D, :], wo_ref[512:D, :], _TN)
        da_slice(6, F - 6 * 256)
        x = x_ref[pl.ds(r0, L), :].astype(f32)
        x1 = x + modv(2) * att
        xhat2, rstd2 = _ln_stats(x1)
        h2 = (xhat2 * (1.0 + modv(4)) + modv(3)).astype(bf16)
        df = df_s[...]
        k0 = math.sqrt(2.0 / math.pi)
        k1 = 0.044715

        def ffn_up(c0, cw):
            cs = slice(c0, c0 + cw)
            u = _dot(h2, w1_ref[cs, :], _NT) + b1_s[:, cs]
            u2 = u * u
            th = jnp.tanh(u * (k0 + (k0 * k1) * u2))
            hp = 0.5 + 0.5 * th
            a = (u * hp).astype(bf16)
            gp = hp + (0.5 * u) * (1.0 - th * th) * (k0 + (3.0 * k0 * k1) * u2)
            ks = range(c0 // 256, (c0 + cw + 255) // 256)
            da = jnp.concatenate(
                [da_s[k, :, 0:min(256, F - 256 * k)] for k in ks], axis=1)
            duf = da * gp
            ab1_s[:, cs] += _colsum8(duf)
            return a, duf.astype(bf16)

        def ffn_dw(c0, cw, a, du):
            cs = slice(c0, c0 + cw)
            v2 = aw2_s[cs, :] + _dot(a, df, _TN)
            aw2_s[cs, :] = v2
            dw2_v[cs, :] = v2.astype(bf16)
            v1 = aw1_s[cs, :] + _dot(du, h2, _TN)
            aw1_s[cs, :] = v1
            dw1_v[cs, :] = v1.astype(bf16)

        facc = None
        dh2 = None
        ups = [ffn_up(*FCHUNKS[0])]
        for ci, (c0, cw) in enumerate(FCHUNKS):
            cs = slice(c0, c0 + cw)
            if ci + 1 < len(FCHUNKS):
                ups.append(ffn_up(*FCHUNKS[ci + 1]))
            a, du = ups[ci]
            t1 = _dot(du, w1_ref[cs, :], _NN)
            dh2 = t1 if dh2 is None else dh2 + t1
            t2 = _dot(a, w2_ref[cs, :], _NN)
            facc = t2 if facc is None else facc + t2
            if ci < len(FCHUNKS) - 2:
                ffn_dw(c0, cw, a, du)
        for ci in range(len(FCHUNKS) - 2, len(FCHUNKS)):
            ffn_dw(*FCHUNKS[ci], *ups[ci])
        av = [avec_s[k] for k in range(2, 6)]
        b2 = b2_s[...]
        datts = []
        for rb in range(0, L, RB):
            rs = slice(rb, rb + RB)
            rows = pl.ds(pl.multiple_of(r0 + rb, RB), RB)
            gout = g_ref[rows, :].astype(f32)
            ff = facc[rs] + b2
            dh = dh2[rs]
            av[3] = av[3] + _colsum8(gout * ff)
            av[2] = av[2] + _colsum8(dh * xhat2[rs])
            av[1] = av[1] + _colsum8(dh)
            dx1 = gout + _ln_bwd(dh * (1.0 + modv(4)), xhat2[rs], rstd2[rs])
            dx1_s[rs, :] = dx1
            out_v[rows, :] = (x1[rs] + modv(5) * ff).astype(bf16)
            av[0] = av[0] + _colsum8(dx1 * att[rs])
            datts.append((dx1 * modv(2)).astype(bf16))
        for k in range(4):
            avec_s[2 + k] = av[k]
        datt = jnp.concatenate(datts, axis=0)
        dot_s[...] = _dot(wo_ref[...], datt, _NT)
        vo = awo_s[...] + _dot(ot_s[...], datt, _NN)
        awo_s[...] = vo
        dwo_v[...] = vo.astype(bf16)
        out_seg(s).start()

        @pl.when(last)
        def _():
            o_dw1.start()
            o_dw2.start()
            o_dwo.start()
            dwmod_cols(2, 6)
            o_dwmod1.start()

        def bwd_group(g):
            g0 = pl.multiple_of(g * GR, 16)
            do = dot_s[pl.ds(g0, GR), :]
            adot = adot_s[pl.ds(g0, GR), :]
            gt = jnp.concatenate([gate_s[pl.ds(g0, GR), :]] * NT, axis=1)
            linv = linv_s[g]
            qt = qkv_s[s, 0, pl.ds(g0, GR), :]
            kt = qkv_s[s, 1, pl.ds(g0, GR), :]
            dop = ((1.0 - gt) * do
                   * _expand([linv[8 * j:8 * j + 8] for j in range(4)])).astype(bf16)
            dopf = dop.astype(f32)
            deltas = _head_sums(dopf * adot)
            rhs = []
            for j in range(4):
                dw = jnp.where(inh[j], dopf[16 * j:16 * j + 32], 0.0).astype(bf16)
                nd = -deltas[j]
                nd_hi = nd.astype(bf16).astype(f32)
                drow = jnp.where(r16 == 0, nd_hi,
                                 jnp.where(r16 == 1, nd - nd_hi, 0.0)).astype(bf16)
                pieces = []
                if j > 0:
                    pieces.append(jnp.zeros((16 * j, L), bf16))
                pieces.append(dw)
                if j < 3:
                    pieces.append(jnp.zeros((48 - 16 * j, L), bf16))
                pieces.append(drow)
                pieces.append(jnp.zeros((32, L), bf16))
                rhs.append(jnp.concatenate(pieces, axis=0))
            rt = [jnp.concatenate([rhs[j][:, 128 * t:128 * (t + 1)] for j in range(4)], axis=1)
                  for t in range(NT)]
            kw = [kt[16 * j:16 * j + 32] for j in range(4)]
            qw = [qt[16 * j:16 * j + 32] for j in range(4)]
            dow = [dop[16 * j:16 * j + 32] for j in range(4)]
            dq_t = [[None] * NT for _ in range(4)]
            dk_t = [[None] * NT for _ in range(4)]
            dv_t = [[None] * NT for _ in range(4)]
            mem_out = {}

            def acc(lst, k, val):
                lst[k] = val if lst[k] is None else lst[k] + val

            def f_dp(t, u):
                e0 = EOFF[t] + 128 * u
                dp = _dot(vtm_s[s, g, 128 * u:128 * (u + 1), :], rt[t], _NN)
                ds = e_s[g, e0:e0 + 128, :].astype(f32) * dp
                return [ds[:, 128 * j:128 * (j + 1)].astype(bf16) for j in range(4)]

            def f_dv(t, u):
                e0 = EOFF[t] + 128 * u
                for j in range(4):
                    e = e_s[g, e0:e0 + 128, 128 * j:128 * (j + 1)]
                    acc(dv_t[j], u, _dot(dow[j][:, 128 * t:128 * (t + 1)], e, _NT))

            def f_dqk(t, u, ds):
                for j in range(4):
                    acc(dk_t[j], u, _dot(qw[j][:, 128 * t:128 * (t + 1)], ds[j], _NT))
                for j in range(4):
                    acc(dq_t[j], t, _dot(kw[j][:, 128 * u:128 * (u + 1)], ds[j], _NN))

            def f_mem(step):
                m = mem_out
                if step == 0:
                    m['dmt'] = dmt_s[g]
                    m['dmtb'] = m['dmt'].astype(bf16)
                    vt = qkv_s[s, 2, pl.ds(g0, GR), :]
                    vx = jnp.concatenate([vt, jnp.ones((16, L), bf16)], axis=0)
                    kf = kt.astype(f32)
                    m['pkf'] = _phi(kf)
                    m['dk'] = (_dot(m['dmtb'], vx, _TN)
                               * jnp.where(kf > 0, 1.0, m['pkf']))
                elif step == 1:
                    m['dv'] = _dot(m['dmtb'][0:GR], m['pkf'].astype(bf16), _NN)
                    amem = amem_s[s, pl.ds(g0, GR), :]
                    adg_s[pl.ds(g0, GR), :] += _lane_fold(do * (amem - adot))
                    dinv = dinv_s[s, g]
                    dnum = gt * do * _expand([dinv[8 * j:8 * j + 8] for j in range(4)])
                    dds = _head_sums(dnum * amem)
                    dden = jnp.zeros((16, L), f32)
                    for j in range(4):
                        dden = jnp.where(r16 == j, -dds[j], dden)
                    m['dnx'] = jnp.concatenate([dnum, dden], axis=0).astype(bf16)
                elif step == 2:
                    qf = qt.astype(f32)
                    m['pqf'] = _phi(qf)
                    m['dq'] = (_dot(mt_s[s, g].astype(bf16), m['dnx'], _TN)
                               * jnp.where(qf > 0, 1.0, m['pqf']))
                else:
                    upd = _dot(m['dnx'], m['pqf'].astype(bf16), _NT)
                    dmt_s[g] = m['dmt'] + jnp.where(mem_mask, upd, 0.0)

            def f_fin():
                def mg(lst):
                    return _merge([jnp.concatenate(lst[j], axis=1)[los[j]:los[j] + 24]
                                   for j in range(4)])

                dqkv_s[0, pl.ds(g0, GR), :] = (mg(dq_t) * SCALE + mem_out['dq']).astype(bf16)
                dqkv_s[1, pl.ds(g0, GR), :] = (mg(dk_t) * SCALE + mem_out['dk']).astype(bf16)
                dqkv_s[2, pl.ds(g0, GR), :] = (mg(dv_t) + mem_out['dv']).astype(bf16)

            return f_dp, f_dv, f_dqk, f_mem, f_fin

        def attn_bwd(p, cc):
            tl = [(t, u) for t in range(NT) for u in range(t + 1)]
            nt = len(tl)
            grp = [bwd_group(BWD_UNROLL * p)]
            dss = {}
            for k in range(BWD_UNROLL * nt + BWD_LAG):
                if k < BWD_UNROLL * nt:
                    gi, ti = divmod(k, nt)
                    if ti == 6 and gi + 1 < BWD_UNROLL:
                        grp.append(bwd_group(BWD_UNROLL * p + gi + 1))
                    dss[k] = grp[gi][0](*tl[ti])
                    grp[gi][1](*tl[ti])
                    if ti in MEM_STEPS:
                        grp[gi][3](MEM_STEPS.index(ti))
                if k >= BWD_LAG:
                    gi, ti = divmod(k - BWD_LAG, nt)
                    grp[gi][2](*tl[ti], dss.pop(k - BWD_LAG))
                    if ti == nt - 1:
                        grp[gi][4]()
            return cc

        with jax.named_scope('attn_bwd'):
            lax.fori_loop(0, NG // BWD_UNROLL, attn_bwd, 0)

        h1 = h1_s[s]

        def dw_proj(idx):
            v = awqkv_s[idx] + _dot(h1, dqkv_s[idx], _NT)
            awqkv_s[idx] = v
            dwqkv_v[idx] = v.astype(bf16)

        HL = L // 2

        def dh1_half(hf):
            acc1 = None
            for idx in range(3):
                t1 = _dot(dqkv_s[idx, :, hf * HL:(hf + 1) * HL], wqkv_ref[idx], _TN)
                acc1 = t1 if acc1 is None else acc1 + t1
            return acc1

        def ln1_bwd(hf, dh1):
            a0 = avec_s[0]
            a1 = avec_s[1]
            for rb in range(0, HL, RB):
                rows = pl.ds(pl.multiple_of(r0 + hf * HL + rb, RB), RB)
                xhat, rstd = _ln_stats(x_ref[rows, :].astype(f32))
                dh = dh1[rb:rb + RB]
                a1 = a1 + _colsum8(dh * xhat)
                a0 = a0 + _colsum8(dh)
                dx = (dx1_s[hf * HL + rb:hf * HL + rb + RB, :]
                      + _ln_bwd(dh * (1.0 + modv(1)), xhat, rstd))
                dx_v[rows, :] = dx.astype(bf16)
            avec_s[0] = a0
            avec_s[1] = a1

        dh1a = dh1_half(0)
        dh1b = dh1_half(1)
        ln1_bwd(0, dh1a)
        dw_proj(0)
        ln1_bwd(1, dh1b)
        dwmod_cols(0, 2)
        dx_seg(s).start()

        @pl.when(last)
        def _():
            o_dwqkv[0].start()
            o_dwmod0.start()

        dw_proj(1)

        @pl.when(last)
        def _():
            o_dwqkv[1].start()

        dw_proj(2)
        return carry

    with jax.named_scope('phase2'):
        lax.fori_loop(0, NSEG, phase2, 0)

    o_dwqkv[2].start()
    rr = _rows((16, D))
    dsc = jnp.zeros((16, D), f32)
    for i in range(6):
        dm = jnp.sum(avec_s[i], axis=0, keepdims=True)
        hi_p = dm.astype(bf16).astype(f32)
        lhs = jnp.where(rr == 0, hi_p, jnp.where(rr == 1, dm - hi_p, 0.0)).astype(bf16)
        dsc = dsc + _dot(lhs, wmod_ref[:, i * D:(i + 1) * D], _NT)
    db1_ref[...] = jnp.sum(ab1_s[...], axis=0).astype(bf16)
    db2_ref[...] = jnp.sum(avec_s[6], axis=0).astype(bf16)
    dgc = jnp.sum(adg_s[...], axis=1, keepdims=True)
    dg = jnp.sum(jnp.where(hsel, dgc, 0.0), axis=0, keepdims=True)
    dbeta_ref[...] = (dg * gate * (1.0 - gate)).astype(bf16)
    dsilu = sig_c * (1.0 + c * (1.0 - sig_c))
    dc_ref[...] = ((dsc[0:1] + dsc[1:2]) * dsilu).astype(bf16)
    for s in range(NSEG):
        out_seg(s).wait()
        dx_seg(s).wait()
    for d in o_dwqkv + [o_dwo, o_dw1, o_dw2, o_dwmod0, o_dwmod1]:
        d.wait()


@jax.jit
def pallas_adaLN_cond__memory_aug_infini_attn__dense_activation_gelu__prompt_kernel(
    A_x: jax.Array,
    A_wq: jax.Array,
    A_wk: jax.Array,
    A_wv: jax.Array,
    A_wo: jax.Array,
    A_beta: jax.Array,
    B_x: jax.Array,
    B_w1: jax.Array,
    B_b1: jax.Array,
    B_w2: jax.Array,
    B_b2: jax.Array,
    c: jax.Array,
    w_mod: jax.Array,
    grad_out: jax.Array,
):
    sd = jax.ShapeDtypeStruct
    out_shape = (
        sd((S, D), bf16), sd((S, D), bf16),
        sd((D, D), bf16), sd((D, D), bf16), sd((D, D), bf16), sd((D, D), bf16),
        sd((F, D), bf16), sd((F, D), bf16), sd((D, 6 * D), bf16),
        sd((1, H), bf16), sd((F,), bf16), sd((D,), bf16), sd((1, D), bf16),
    )
    vm = pltpu.VMEM
    scratch = [
        vm((S, D), bf16), vm((S, D), bf16), vm((3, D, D), bf16), vm((D, D), bf16),
        vm((F, D), bf16), vm((F, D), bf16), vm((D, 6 * D), bf16),
        vm((3, D, D), bf16), vm((D, D), bf16),
        vm((F, D), bf16), vm((F, D), bf16), vm((D, 6 * D), bf16),
        vm((16, 6 * D), f32),
        vm((D, 128), f32),
        vm((NSEG, D, L), bf16),
        vm((NSEG, 3, D, L), bf16),
        vm((NSEG, NG, L, 128), bf16),
        vm((NSEG, NG, L, 128), bf16),
        vm((NSEG, NG, 96, GR), f32),
        vm((NG, 96, GR), f32),
        vm((NG, EROWS, 512), bf16),
        vm((EROWS, 512), f32), vm((EROWS, 512), f32),
        vm((NT, 8, 512), f32), vm((NT, 8, 512), f32),
        vm((NG, 32, L), f32),
        vm((NSEG, NG, 32, L), f32),
        vm((D, L), f32),
        vm((NSEG, D, L), f32),
        vm((D, L), bf16),
        vm((D, L), f32),
        vm((3, D, L), bf16),
        vm((L, D), f32),
        vm((3, D, D), f32), vm((D, D), f32), vm((F, D), f32), vm((F, D), f32),
        vm((7, 8, D), f32), vm((8, F), f32), vm((D, 128), f32),
        vm((7, L, 256), f32), vm((L, D), bf16), vm((D, 128), f32),
        vm((1, F), f32), vm((1, D), f32),
        pltpu.SemaphoreType.DMA((12,)), pltpu.SemaphoreType.DMA((16,)),
    ]
    hbm = pl.BlockSpec(memory_space=pl.ANY)
    vmem = pl.BlockSpec(memory_space=pltpu.VMEM)
    outs = pl.pallas_call(
        _kernel,
        out_shape=out_shape,
        in_specs=[hbm] * 9 + [vmem] * 4,
        out_specs=tuple([hbm] * 9 + [vmem] * 4),
        scratch_shapes=scratch,
        compiler_params=pltpu.CompilerParams(vmem_limit_bytes=125 * 1024 * 1024),
    )(A_x.reshape(S, D), grad_out.reshape(S, D), A_wq, A_wk, A_wv, A_wo, B_w1.T, B_w2, w_mod,
      A_beta.reshape(1, H), B_b1, B_b2, c)
    (out, dx, dwq, dwk, dwv, dwo, dw1t, dw2, dwmod, dbeta, db1, db2, dc) = outs
    return (out.reshape(1, S, D), dx.reshape(1, S, D), dwq, dwk, dwv, dwo,
            dbeta.reshape(H), dw1t.T, db1, dw2, db2, dc, dwmod)
```

```python
import math

import jax
import jax.numpy as jnp
from jax import lax
import jax.experimental.pallas as pl
import jax.experimental.pallas.tpu as pltpu

S, D, H, DH, NSEG, L, F = 2048, 640, 32, 20, 4, 512, 1728
GR = 80
NG = D // GR
NT = L // 128
EROWS = 128 * NT * (NT + 1) // 2
EOFF = [128 * t * (t + 1) // 2 for t in range(NT)]
SCALE = DH ** (-0.5)
LOG2E = math.log2(math.e)
LN_EPS = 1e-5
DEN_EPS = 1e-6
NEG = -1e30
BWD_UNROLL = 4
BWD_LAG = 2
RB = 64
RB2 = 128
MEM_STEPS = (2, 5, 7, 9)
FT = 1536
FCHUNKS = [(0, 512), (512, 512), (1024, 512), (1536, 192)]

f32 = jnp.float32
bf16 = jnp.bfloat16

_NN = (((1,), (0,)), ((), ()))
_NT = (((1,), (1,)), ((), ()))
_TN = (((0,), (0,)), ((), ()))
_TT = (((0,), (1,)), ((), ()))


def _dot(a, b, dn):
    return lax.dot_general(a, b, dn, preferred_element_type=f32)


def _phi(t):
    return jnp.where(t > 0, t + 1.0, jnp.exp(t))


def _rows(shape):
    return lax.broadcasted_iota(jnp.int32, shape, 0)


def _cols(shape):
    return lax.broadcasted_iota(jnp.int32, shape, 1)


def _merge(parts):
    n = parts[0].shape[1]
    lo = _rows((8, n)) < 4
    a0, a1, a2, a3 = parts
    return jnp.concatenate([
        a0[0:16], jnp.where(lo, a0[16:24], a1[0:8]), a1[8:24],
        a2[0:16], jnp.where(lo, a2[16:24], a3[0:8]), a3[8:24]], axis=0)


def _expand(tiles):
    n = tiles[0].shape[1]
    lo = _rows((8, n)) < 4
    t0, t1, t2, t3 = tiles
    return jnp.concatenate([
        t0, t0, jnp.where(lo, t0, t1), t1, t1,
        t2, t2, jnp.where(lo, t2, t3), t3, t3], axis=0)


def _head_sums(a):
    n = a.shape[1]
    lo = _rows((8, n)) < 4
    z = jnp.zeros((8, n), a.dtype)
    p = [
        a[0:8] + a[8:16] + jnp.where(lo, a[16:24], z),
        jnp.where(lo, z, a[16:24]) + a[24:32] + a[32:40],
        a[40:48] + a[48:56] + jnp.where(lo, a[56:64], z),
        jnp.where(lo, z, a[56:64]) + a[64:72] + a[72:80],
    ]
    return [jnp.sum(t, axis=0, keepdims=True) for t in p]


def _rot64(a):
    return pltpu.roll(a, 64, 1)


def _pair_window(wa, wb):
    left = _cols((16, 128)) < 64
    ra = _rot64(wa)
    return jnp.concatenate([
        jnp.where(left, ra[0:16], 0.0), jnp.where(left, ra[16:32], wb[0:16]),
        jnp.where(left, 0.0, wb[16:32])], axis=0)


def _unpack_pairs(a):
    p0, p1 = a[:, 0:128], a[:, 128:256]
    return jnp.concatenate([_rot64(p0), p0, _rot64(p1), p1], axis=1)


def _lane_fold(a):
    return (a[:, 0:128] + a[:, 128:256]) + (a[:, 256:384] + a[:, 384:512])


def _ln_stats(x):
    mu = jnp.mean(x, axis=-1, keepdims=True)
    xc = x - mu
    var = jnp.mean(xc * xc, axis=-1, keepdims=True)
    rstd = lax.rsqrt(var + LN_EPS)
    return xc * rstd, rstd


def _ln_bwd(dxhat, xhat, rstd):
    m1 = jnp.mean(dxhat, axis=-1, keepdims=True)
    m2 = jnp.mean(dxhat * xhat, axis=-1, keepdims=True)
    return rstd * (dxhat - m1 - xhat * m2)


def _colsum8(a):
    r, n = a.shape
    return jnp.sum(a.reshape(r // 8, 8, n), axis=0)


def _kernel(x_hbm, g_hbm, wq_hbm, wk_hbm, wv_hbm, wo_hbm, w1_hbm, w2_hbm, wmod_hbm,
            beta_ref, b1_ref, b2_ref, c_ref,
            out_hbm, dx_hbm, dwq_hbm, dwk_hbm, dwv_hbm, dwo_hbm, dw1_hbm, dw2_hbm, dwmod_hbm,
            dbeta_ref, db1_ref, db2_ref, dc_ref,
            x_ref, g_ref, wqkv_ref, wo_ref, w1_ref, w2_ref, wmod_ref,
            dwqkv_v, dwo_v, dw1_v, dw2_v, dwmod_v,
            mod_s, gate_s, h1_s, qkv_s, ktm_s, vtm_s, mt_s, dmt_s, e_s, st0, st1, m0, m1,
            linv_s, dinv_s, adot_s, amem_s, ot_s, dot_s, dqkv_s, dx1_s,
            awqkv_s, awo_s, aw1_s, aw2_s, avec_s, ab1_s, adg_s, da_s, df_s, sccol_s, b1_s, b2_s, b1t_s, ab1t_s,
            isem, osem):
    out_v = g_ref
    dx_v = x_ref
    st_s = (st0, st1)
    m_s = (m0, m1)

    def cp(src, dst, sem):
        return pltpu.make_async_copy(src, dst, sem)

    in_wmod0 = cp(wmod_hbm.at[:, 0:2 * D], wmod_ref.at[:, 0:2 * D], isem.at[0])
    in_x0 = cp(x_hbm.at[0:L], x_ref.at[0:L], isem.at[1])
    in_wq = cp(wq_hbm, dwqkv_v.at[0], isem.at[2])
    in_wk = cp(wk_hbm, dwqkv_v.at[1], isem.at[3])
    in_wv = cp(wv_hbm, dwqkv_v.at[2], isem.at[4])
    in_x1 = cp(x_hbm.at[L:2 * L], x_ref.at[L:2 * L], isem.at[5])
    in_x2 = cp(x_hbm.at[2 * L:S], x_ref.at[2 * L:S], isem.at[11])
    in_wmod1 = cp(wmod_hbm.at[:, 2 * D:6 * D], wmod_ref.at[:, 2 * D:6 * D], isem.at[6])
    in_wo = cp(wo_hbm, wo_ref, isem.at[7])
    in_w1 = cp(w1_hbm, w1_ref, isem.at[8])
    in_w2 = cp(w2_hbm, w2_ref, isem.at[9])
    in_g = cp(g_hbm, g_ref, isem.at[10])

    def out_seg(s):
        r0 = pl.multiple_of(s * L, L)
        return cp(out_v.at[pl.ds(r0, L)], out_hbm.at[pl.ds(r0, L)], osem.at[s])

    def dx_seg(s):
        r0 = pl.multiple_of(s * L, L)
        return cp(dx_v.at[pl.ds(r0, L)], dx_hbm.at[pl.ds(r0, L)], osem.at[NSEG + s])

    o_dwqkv = [cp(dwqkv_v.at[i], dst, osem.at[8 + i])
               for i, dst in enumerate((dwq_hbm, dwk_hbm, dwv_hbm))]
    o_dwo = cp(dwo_v, dwo_hbm, osem.at[11])
    o_dw1 = cp(dw1_v, dw1_hbm, osem.at[12])
    o_dw2 = cp(dw2_v, dw2_hbm, osem.at[13])
    o_dwmod0 = cp(dwmod_v.at[:, 0:2 * D], dwmod_hbm.at[:, 0:2 * D], osem.at[14])
    o_dwmod1 = cp(dwmod_v.at[:, 2 * D:6 * D], dwmod_hbm.at[:, 2 * D:6 * D], osem.at[15])

    for d in (in_wmod0, in_x0, in_wk, in_wv):
        d.start()
    for r in (awo_s, avec_s, ab1_s, ab1t_s, adg_s, dmt_s, awqkv_s, aw1_s, aw2_s):
        r[...] = jnp.zeros(r.shape, r.dtype)
    mt_s[0] = jnp.zeros(mt_s.shape[1:], f32)
    c = c_ref[...].astype(f32)
    sig_c = jax.nn.sigmoid(c)
    silu_c = c * sig_c
    silu8 = jnp.broadcast_to(silu_c, (16, D)).astype(bf16)
    gate = jax.nn.sigmoid(beta_ref[...].astype(f32))
    hsel = (_rows((D, H)) // DH) == _cols((D, H))
    gcol = jnp.sum(jnp.where(hsel, gate, 0.0), axis=1, keepdims=True)
    gate_s[...] = jnp.broadcast_to(gcol, (D, 128))
    sccol_s[...] = jnp.broadcast_to(silu_c, (128, D)).T
    b1_s[...] = b1_ref[...].astype(f32).reshape(1, F)
    b2_s[...] = b2_ref[...].astype(f32).reshape(1, D)
    b1t_s[...] = jnp.concatenate(
        [jnp.broadcast_to(b1_s[:, FT:F], (128, F - FT)),
         jnp.zeros((128, 256 - (F - FT)), f32)], axis=1).T[0:F - FT]
    in_wmod0.wait()
    in_wq.start()
    in_x1.start()
    mod_s[:, 0:2 * D] = _dot(silu8, wmod_ref[:, 0:2 * D], _NN)
    in_x0.wait()

    def modv(i):
        return mod_s[0:1, i * D:(i + 1) * D]

    mr = _rows((96, GR))
    mc = _cols((96, GR)) // DH
    mem_mask = jnp.where(mr < GR, mr // DH, mr - GR) == mc

    def ln1_fwd(s):
        xhat, _ = _ln_stats(x_ref[s * L:(s + 1) * L, :].astype(f32))
        h1_s[s] = (xhat * (1.0 + modv(1)) + modv(0)).T.astype(bf16)

    def proj(idx, s):
        if s == 0:
            w = dwqkv_v[idx]
            wqkv_ref[idx] = w.T
            return _dot(w, h1_s[s], _TN)
        return _dot(wqkv_ref[idx], h1_s[s], _NN)

    def proj_k(s):
        kt = proj(1, s)
        qkv_s[s, 1] = kt.astype(bf16)
        for g in range(NG):
            ktm_s[s, g] = jnp.concatenate(
                [kt[g * GR:(g + 1) * GR] * (SCALE * LOG2E), jnp.zeros((48, L), f32)],
                axis=0).T.astype(bf16)

    def proj_v(s):
        vt = proj(2, s)
        qkv_s[s, 2] = vt.astype(bf16)
        for g in range(NG):
            vtm_s[s, g] = jnp.concatenate(
                [vt[g * GR:(g + 1) * GR], jnp.ones((16, L), f32), jnp.zeros((32, L), f32)],
                axis=0).T.astype(bf16)

    def proj_q(s):
        qt = proj(0, s)
        qkv_s[s, 0] = qt.astype(bf16)

    def mem_upd(s):
        ones = jnp.ones((16, L), bf16)
        for g in range(NG):
            rs = slice(g * GR, (g + 1) * GR)
            pk = _phi(qkv_s[s, 1, rs, :].astype(f32)).astype(bf16)
            vx = jnp.concatenate([qkv_s[s, 2, rs, :], ones], axis=0)
            upd = _dot(vx, pk, _NT)
            mt_s[s + 1, g] = mt_s[s, g] + jnp.where(mem_mask, upd, 0.0)

    def mem_read(s):
        for g in range(NG):
            rs = slice(g * GR, (g + 1) * GR)
            pq = _phi(qkv_s[s, 0, rs, :].astype(f32)).astype(bf16)
            numx = _dot(mt_s[s, g].astype(bf16), pq, _NN)
            dinvs = [jnp.broadcast_to(1.0 / (numx[GR + j:GR + j + 1] + DEN_EPS), (8, L))
                     for j in range(4)]
            dinv_s[s, g] = jnp.concatenate(dinvs, axis=0)
            amem_s[s, rs, :] = numx[0:GR] * _expand(dinvs)

    ln1_fwd(0)
    in_wk.wait()
    with jax.named_scope('phase1'):
        proj_k(0)
        in_wv.wait()
        in_x2.start()
        for s in range(NSEG):
            if s == 1:
                in_x2.wait()
                for d in (in_wmod1, in_g, in_w2, in_wo, in_w1):
                    d.start()
            if s > 0:
                proj_k(s)
                mem_read(s - 1)
            if s + 1 < NSEG:
                proj_v(s)
                if s == 0:
                    in_wq.wait()
                    in_x1.wait()
                ln1_fwd(s + 1)
                proj_q(s)
                mem_upd(s)
            else:
                proj_q(s)
                proj_v(s)
                mem_read(s)

    in_wmod1.wait()
    mod_s[:, 2 * D:6 * D] = _dot(silu8, wmod_ref[:, 2 * D:6 * D], _NN)
    for d in (in_wo, in_w1, in_w2, in_g):
        d.wait()

    causal_t = _rows((64, 128)) <= _cols((64, 128))
    causal_t = jnp.concatenate([causal_t] * 4, axis=1)
    causal_b = _rows((64, 128)) <= (_cols((64, 128)) & 63)
    causal_b = jnp.concatenate([causal_b] * 2, axis=1)
    upper8 = jnp.concatenate([_cols((8, 128)) >= 64] * 4, axis=1)
    upper64 = jnp.concatenate([upper8] * 8, axis=0)
    wrow = _rows((32, L))
    r16 = _rows((16, L))
    inh = [(wrow >= 4 * j) & (wrow < 4 * j + DH) for j in range(4)]
    los = (0, 0, 8, 8)

    def dwmod_cols(lo, hi):
        sc_col = jnp.concatenate([sccol_s[...]] * (D // 128), axis=1)
        for i in range(lo, hi):
            dm = jnp.sum(avec_s[i], axis=0, keepdims=True)
            dwmod_v[:, i * D:(i + 1) * D] = (sc_col * dm).astype(bf16)

    def make_df(s, valid):
        gsum = None
        for rb in range(0, L, 64):
            gout = g_ref[pl.ds(pl.multiple_of(s * L + rb, 64), 64), :].astype(f32)
            df_s[rb:rb + 64, :] = (gout * (0.5 * modv(5))).astype(bf16)
            gsum = _colsum8(gout) if gsum is None else gsum + _colsum8(gout)
        avec_s[6] += jnp.where(valid, gsum, 0.0)

    make_df(NSEG - 1, True)

    def epilogue():
        o_dwqkv[2].start()
        rr = _rows((16, D))
        dsc = jnp.zeros((16, D), f32)
        for i in range(6):
            dm = jnp.sum(avec_s[i], axis=0, keepdims=True)
            hi_p = dm.astype(bf16).astype(f32)
            lhs = jnp.where(rr == 0, hi_p, jnp.where(rr == 1, dm - hi_p, 0.0)).astype(bf16)
            dsc = dsc + _dot(lhs, wmod_ref[:, i * D:(i + 1) * D], _NT)
        ab1_s[:, FT:F] = _colsum8(ab1t_s[...].T)[:, 0:F - FT]
        db1_ref[...] = jnp.sum(ab1_s[...], axis=0).astype(bf16)
        db2_ref[...] = jnp.sum(avec_s[6] * modv(5), axis=0).astype(bf16)
        dgc = jnp.sum(adg_s[...], axis=1, keepdims=True)
        dg = jnp.sum(jnp.where(hsel, dgc, 0.0), axis=0, keepdims=True)
        dbeta_ref[...] = (dg * gate * (1.0 - gate)).astype(bf16)
        dsilu = sig_c * (1.0 + c * (1.0 - sig_c))
        dc_ref[...] = ((dsc[0:1] + dsc[1:2]) * dsilu).astype(bf16)
        for s in range(NSEG):
            out_seg(s).wait()
            dx_seg(s).wait()
        for d in o_dwqkv + [o_dwo, o_dw1, o_dw2, o_dwmod0, o_dwmod1]:
            d.wait()

    def phase2(i, carry):
        s = NSEG - 1 - i
        r0 = pl.multiple_of(s * L, L)
        last = i == NSEG - 1

        def a_prep(g):
            g0 = pl.multiple_of(g * GR, 16)
            qs = qkv_s[s, 0, pl.ds(g0, GR), :]
            rhs, qws = [], []
            for j in range(4):
                qw = jnp.where(inh[j], qs[16 * j:16 * j + 32].astype(f32), 0.0)
                qws.append(qw)
                pieces = []
                if j > 0:
                    pieces.append(jnp.zeros((16 * j, L), bf16))
                pieces.append(qw.astype(bf16))
                pieces.append(jnp.zeros((96 - 16 * j, L), bf16))
                rhs.append(jnp.concatenate(pieces, axis=0))
            return rhs, qws

        def a_tile(g, prep, slot, t):
            rhs, qws = prep
            n = 128 * (t + 1)
            cs = slice(128 * t, n)
            r = jnp.concatenate([rhs[j][:, cs] for j in range(4)], axis=1)
            st = _dot(ktm_s[s, g, 0:n - 64, :], r, _NN)
            w0 = _pair_window(qws[0][:, cs], qws[1][:, cs]).astype(bf16)
            w1 = _pair_window(qws[2][:, cs], qws[3][:, cs]).astype(bf16)
            rp = jnp.concatenate([
                jnp.concatenate([w0, jnp.zeros((80, 128), bf16)], axis=0),
                jnp.concatenate([jnp.zeros((32, 128), bf16), w1, jnp.zeros((48, 128), bf16)],
                                axis=0)], axis=1)
            bot = jnp.where(causal_b, _dot(ktm_s[s, g, n - 64:n, :], rp, _NN), NEG)
            diag = jnp.where(causal_t, st[n - 128:n - 64], NEG)
            st = jnp.concatenate([st[0:n - 128], diag], axis=0) if t > 0 else diag
            st_s[slot][EOFF[t]:EOFF[t] + n - 64, :] = st
            st_s[slot][EOFF[t] + n - 64:EOFF[t] + n, 0:256] = bot
            mb = jnp.broadcast_to(jnp.max(bot, axis=0, keepdims=True), (8, 256))
            mt = jnp.broadcast_to(jnp.max(st, axis=0, keepdims=True), (8, 512))
            mx = jnp.where(upper8, jnp.maximum(mt, _unpack_pairs(mb)), mt)
            m_s[slot][t, 0:8, :] = mx
            m_s[slot][t, 8:16, 0:256] = jnp.concatenate(
                [jnp.where(upper8[:, 0:128], mx[:, 128 * (j + 1):128 * (j + 2)],
                           _rot64(mx[:, 128 * j:128 * (j + 1)])) for j in (0, 2)], axis=1)

        def b_prep(g):
            g0 = pl.multiple_of(g * GR, 16)
            vt = qkv_s[s, 2, pl.ds(g0, GR), :]
            return [jnp.where(inh[j], vt[16 * j:16 * j + 32].astype(f32), 1.0).astype(bf16)
                    for j in range(4)]

        def b_tile(g, vws, slot, t):
            n = 128 * (t + 1)
            e32 = jnp.exp2(st_s[slot][EOFF[t]:EOFF[t] + n - 64, :] - m_s[slot][t, 0:1, :])
            eb = jnp.exp2(st_s[slot][EOFF[t] + n - 64:EOFF[t] + n, 0:256]
                          - m_s[slot][t, 8:9, 0:256])
            e32 = jnp.concatenate([e32, jnp.where(upper64, _unpack_pairs(eb), 0.0)], axis=0)
            e_s[g, EOFF[t]:EOFF[t] + n, :] = e32.astype(bf16)
            return [_dot(vws[j][:, 0:n], e32[:, 128 * j:128 * (j + 1)].astype(bf16), _NN)
                    for j in range(4)]

        def b_fin(g, pv):
            g0 = pl.multiple_of(g * GR, 16)
            parts, linvs = [], []
            for j in range(4):
                ow = jnp.concatenate([pv[t][j] for t in range(NT)], axis=1)
                linv = 1.0 / (ow[24:32] if j < 2 else ow[0:8])
                linvs.append(linv)
                parts.append(ow[los[j]:los[j] + 24] * jnp.concatenate([linv] * 3, axis=0))
            adot = _merge(parts)
            linv_s[g] = jnp.concatenate(linvs, axis=0)
            adot_s[pl.ds(g0, GR), :] = adot
            gt = jnp.concatenate([gate_s[pl.ds(g0, GR), :]] * NT, axis=1)
            amem = amem_s[s, pl.ds(g0, GR), :]
            ot_s[pl.ds(g0, GR), :] = (gt * amem + (1.0 - gt) * adot).astype(bf16)

        def da_slice(k, lo, hi):
            c0 = pl.multiple_of(k * 256, 256)
            da_s[k, lo:hi, :] = _dot(df_s[lo:hi, :], w2_ref[pl.ds(c0, 256), :], _NT)

        def ab(g, slot):
            rhs = a_prep(g + 1)
            vws = b_prep(g)
            pv = []
            for t in range(NT):
                a_tile(g + 1, rhs, 1 - slot, t)
                if not (isinstance(g, int) and g == NG - 2):
                    da_slice(g, 128 * t, 128 * (t + 1))
                pv.append(b_tile(g, vws, slot, t))
            b_fin(g, pv)

        def fwd_pair(p, cc):
            ab(2 * p, 0)
            ab(2 * p + 1, 1)
            return cc

        with jax.named_scope('attn_fwd'):
            rhs0 = a_prep(0)
            for t in range(NT):
                a_tile(0, rhs0, 0, NT - 1 - t)
            lax.fori_loop(0, NG // 2 - 1, fwd_pair, 0)
            ab(NG - 2, 0)
            vws = b_prep(NG - 1)
            pv = [b_tile(NG - 1, vws, 1, 0)]
            att = _dot(ot_s[0:256, :], wo_ref[0:256, :], _TN)
            pv += [b_tile(NG - 1, vws, 1, t) for t in range(1, 3)]
            att = att + _dot(ot_s[256:512, :], wo_ref[256:512, :], _TN)
            pv.append(b_tile(NG - 1, vws, 1, 3))
            b_fin(NG - 1, pv)

        att = att + _dot(ot_s[512:D, :], wo_ref[512:D, :], _TN)
        df = df_s[...]
        da_t = _dot(w2_ref[FT:F, :], df, _NT)
        x1s, xhs, rss, h2s = [], [], [], []
        for rb in range(0, L, 64):
            rows = pl.ds(pl.multiple_of(r0 + rb, 64), 64)
            x1b = x_ref[rows, :].astype(f32) + modv(2) * att[rb:rb + 64]
            xh, rsd = _ln_stats(x1b)
            x1s.append(x1b)
            xhs.append(xh)
            rss.append(rsd)
            h2s.append((xh * (1.0 + modv(4)) + modv(3)).astype(bf16))
        x1 = jnp.concatenate(x1s, axis=0)
        xhat2 = jnp.concatenate(xhs, axis=0)
        rstd2 = jnp.concatenate(rss, axis=0)
        h2 = jnp.concatenate(h2s, axis=0)
        k0 = math.sqrt(2.0 / math.pi)
        k1 = 0.044715

        def gelu2(u, da):
            u2 = u * u
            th = jnp.tanh(u * (k0 + (k0 * k1) * u2))
            t1 = 1.0 + th
            a2 = u * t1
            gp = t1 + a2 * (1.0 - th) * (k0 + (3.0 * k0 * k1) * u2)
            return a2.astype(bf16), da * gp

        def ffn_up(c0, cw):
            cs = slice(c0, c0 + cw)
            if c0 == FT:
                u = (_dot(w1_ref[cs, :], h2, _NT)
                     + jnp.concatenate([b1t_s[...]] * NT, axis=1))
                a, duf = gelu2(u, da_t)
                ab1t_s[0:cw, :] += _lane_fold(duf)
                return a, duf.astype(bf16)
            u = _dot(h2, w1_ref[cs, :], _NT) + b1_s[:, cs]
            da = jnp.concatenate([da_s[k] for k in range(c0 // 256, (c0 + cw) // 256)], axis=1)
            a, duf = gelu2(u, da)
            ab1_s[:, cs] += _colsum8(duf)
            return a, duf.astype(bf16)

        def ffn_dw(c0, cw, a, du):
            cs = slice(c0, c0 + cw)
            dn = _NN if c0 == FT else _TN
            v2 = aw2_s[cs, :] + _dot(a, df, dn)
            aw2_s[cs, :] = v2
            dw2_v[cs, :] = v2.astype(bf16)
            v1 = aw1_s[cs, :] + _dot(du, h2, dn)
            aw1_s[cs, :] = v1
            dw1_v[cs, :] = v1.astype(bf16)

        facc = None
        dh2 = None
        ups = [ffn_up(*FCHUNKS[0])]
        for ci, (c0, cw) in enumerate(FCHUNKS):
            cs = slice(c0, c0 + cw)
            if ci + 1 < len(FCHUNKS):
                ups.append(ffn_up(*FCHUNKS[ci + 1]))
            a, du = ups[ci]
            dn = _TN if c0 == FT else _NN
            t1 = _dot(du, w1_ref[cs, :], dn)
            dh2 = t1 if dh2 is None else dh2 + t1
            t2 = _dot(a, w2_ref[cs, :], dn)
            facc = t2 if facc is None else facc + t2
            if ci < len(FCHUNKS) - 2:
                ffn_dw(c0, cw, a, du)
        for ci in range(len(FCHUNKS) - 2, len(FCHUNKS)):
            ffn_dw(*FCHUNKS[ci], *ups[ci])
        av = [avec_s[k] for k in range(2, 6)]
        b2 = b2_s[...]
        datts = []
        for rb in range(0, L, RB2):
            rs = slice(rb, rb + RB2)
            rows = pl.ds(pl.multiple_of(r0 + rb, RB2), RB2)
            gout = g_ref[rows, :].astype(f32)
            ff = 0.5 * facc[rs] + b2
            dh = dh2[rs]
            av[3] = av[3] + _colsum8(gout * ff)
            av[2] = av[2] + _colsum8(dh * xhat2[rs])
            av[1] = av[1] + _colsum8(dh)
            dx1 = gout + _ln_bwd(dh * (1.0 + modv(4)), xhat2[rs], rstd2[rs])
            dx1_s[rs, :] = dx1
            out_v[rows, :] = (x1[rs] + modv(5) * ff).astype(bf16)
            av[0] = av[0] + _colsum8(dx1 * att[rs])
            datts.append((dx1 * modv(2)).astype(bf16))
        for k in range(4):
            avec_s[2 + k] = av[k]
        datt = jnp.concatenate(datts, axis=0)
        dot_s[...] = _dot(wo_ref[...], datt, _NT)
        vo = awo_s[...] + _dot(ot_s[...], datt, _NN)
        awo_s[...] = vo
        dwo_v[...] = vo.astype(bf16)
        out_seg(s).start()

        @pl.when(last)
        def _():
            o_dw1.start()
            o_dw2.start()
            o_dwo.start()
            dwmod_cols(2, 6)
            o_dwmod1.start()

        def bwd_group(g):
            g0 = pl.multiple_of(g * GR, 16)
            do = dot_s[pl.ds(g0, GR), :]
            adot = adot_s[pl.ds(g0, GR), :]
            gt = jnp.concatenate([gate_s[pl.ds(g0, GR), :]] * NT, axis=1)
            linv = linv_s[g]
            qt = qkv_s[s, 0, pl.ds(g0, GR), :]
            kt = qkv_s[s, 1, pl.ds(g0, GR), :]
            dop = ((1.0 - gt) * do
                   * _expand([linv[8 * j:8 * j + 8] for j in range(4)])).astype(bf16)
            dopf = dop.astype(f32)
            deltas = _head_sums(dopf * adot)
            rhs, dws, drows = [], [], []
            for j in range(4):
                dw = jnp.where(inh[j], dopf[16 * j:16 * j + 32], 0.0)
                nd = -deltas[j]
                nd_hi = nd.astype(bf16).astype(f32)
                drow = jnp.where(r16 == 0, nd_hi, jnp.where(r16 == 1, nd - nd_hi, 0.0))
                dws.append(dw)
                drows.append(drow)
                pieces = []
                if j > 0:
                    pieces.append(jnp.zeros((16 * j, L), bf16))
                pieces.append(dw.astype(bf16))
                if j < 3:
                    pieces.append(jnp.zeros((48 - 16 * j, L), bf16))
                pieces.append(drow.astype(bf16))
                pieces.append(jnp.zeros((32, L), bf16))
                rhs.append(jnp.concatenate(pieces, axis=0))
            rt = [jnp.concatenate([rhs[j][:, 128 * t:128 * (t + 1)] for j in range(4)], axis=1)
                  for t in range(NT)]

            def packed_rhs(t):
                cs = slice(128 * t, 128 * (t + 1))
                cols = []
                for j in (0, 2):
                    win = _pair_window(dws[j][:, cs], dws[j + 1][:, cs])
                    dr = jnp.where(_cols((16, 128)) < 64, _rot64(drows[j][:, cs]),
                                   drows[j + 1][:, cs])
                    pieces = [win.astype(bf16), jnp.zeros((32, 128), bf16)]
                    if j:
                        pieces = pieces[::-1]
                    cols.append(jnp.concatenate(
                        pieces + [dr.astype(bf16), jnp.zeros((32, 128), bf16)], axis=0))
                return jnp.concatenate(cols, axis=1)

            kw = [kt[16 * j:16 * j + 32] for j in range(4)]
            qw = [qt[16 * j:16 * j + 32] for j in range(4)]
            dow = [dop[16 * j:16 * j + 32] for j in range(4)]
            dq_t = [[None] * NT for _ in range(4)]
            dk_t = [[None] * NT for _ in range(4)]
            dv_t = [[None] * NT for _ in range(4)]
            mem_out = {}

            def acc(lst, k, val):
                lst[k] = val if lst[k] is None else lst[k] + val

            def f_dp(t, u):
                e0 = EOFF[t] + 128 * u
                if u < t:
                    dp = _dot(vtm_s[s, g, 128 * u:128 * (u + 1), :], rt[t], _NN)
                else:
                    top = _dot(vtm_s[s, g, 128 * u:128 * u + 64, :], rt[t], _NN)
                    bot = _dot(vtm_s[s, g, 128 * u + 64:128 * (u + 1), :], packed_rhs(t), _NN)
                    dp = jnp.concatenate([top, _unpack_pairs(bot)], axis=0)
                ds = e_s[g, e0:e0 + 128, :].astype(f32) * dp
                return [ds[:, 128 * j:128 * (j + 1)].astype(bf16) for j in range(4)]

            def f_dv(t, u):
                e0 = EOFF[t] + 128 * u
                for j in range(4):
                    e = e_s[g, e0:e0 + 128, 128 * j:128 * (j + 1)]
                    acc(dv_t[j], u, _dot(dow[j][:, 128 * t:128 * (t + 1)], e, _NT))

            def f_dqk(t, u, ds):
                for j in range(4):
                    acc(dk_t[j], u, _dot(qw[j][:, 128 * t:128 * (t + 1)], ds[j], _NT))
                for j in range(4):
                    acc(dq_t[j], t, _dot(kw[j][:, 128 * u:128 * (u + 1)], ds[j], _NN))

            def f_mem(step):
                m = mem_out
                if step == 0:
                    m['dmt'] = dmt_s[g]
                    m['dmtb'] = m['dmt'].astype(bf16)
                    vt = qkv_s[s, 2, pl.ds(g0, GR), :]
                    vx = jnp.concatenate([vt, jnp.ones((16, L), bf16)], axis=0)
                    kf = kt.astype(f32)
                    m['pkf'] = _phi(kf)
                    m['dk'] = (_dot(m['dmtb'], vx, _TN)
                               * jnp.where(kf > 0, 1.0, m['pkf']))
                elif step == 1:
                    m['dv'] = _dot(m['dmtb'][0:GR], m['pkf'].astype(bf16), _NN)
                    amem = amem_s[s, pl.ds(g0, GR), :]
                    adg_s[pl.ds(g0, GR), :] += _lane_fold(do * (amem - adot))
                    dinv = dinv_s[s, g]
                    dnum = gt * do * _expand([dinv[8 * j:8 * j + 8] for j in range(4)])
                    dds = _head_sums(dnum * amem)
                    dden = jnp.zeros((16, L), f32)
                    for j in range(4):
                        dden = jnp.where(r16 == j, -dds[j], dden)
                    m['dnx'] = jnp.concatenate([dnum, dden], axis=0).astype(bf16)
                elif step == 2:
                    qf = qt.astype(f32)
                    m['pqf'] = _phi(qf)
                    m['dq'] = (_dot(mt_s[s, g].astype(bf16), m['dnx'], _TN)
                               * jnp.where(qf > 0, 1.0, m['pqf']))
                else:
                    upd = _dot(m['dnx'], m['pqf'].astype(bf16), _NT)
                    dmt_s[g] = m['dmt'] + jnp.where(mem_mask, upd, 0.0)

            def f_fin():
                def mg(lst):
                    return _merge([jnp.concatenate(lst[j], axis=1)[los[j]:los[j] + 24]
                                   for j in range(4)])

                dqkv_s[0, pl.ds(g0, GR), :] = (mg(dq_t) * SCALE + mem_out['dq']).astype(bf16)
                dqkv_s[1, pl.ds(g0, GR), :] = (mg(dk_t) * SCALE + mem_out['dk']).astype(bf16)
                dqkv_s[2, pl.ds(g0, GR), :] = (mg(dv_t) + mem_out['dv']).astype(bf16)

            return f_dp, f_dv, f_dqk, f_mem, f_fin

        def attn_bwd(p, cc):
            tl = [(t, u) for t in range(NT) for u in range(t + 1)]
            nt = len(tl)
            grp = [bwd_group(BWD_UNROLL * p)]
            dss = {}
            for k in range(BWD_UNROLL * nt + BWD_LAG):
                if k < BWD_UNROLL * nt:
                    gi, ti = divmod(k, nt)
                    if ti == 6 and gi + 1 < BWD_UNROLL:
                        grp.append(bwd_group(BWD_UNROLL * p + gi + 1))
                    dss[k] = grp[gi][0](*tl[ti])
                    grp[gi][1](*tl[ti])
                    if ti in MEM_STEPS:
                        grp[gi][3](MEM_STEPS.index(ti))
                if k >= BWD_LAG:
                    gi, ti = divmod(k - BWD_LAG, nt)
                    grp[gi][2](*tl[ti], dss.pop(k - BWD_LAG))
                    if ti == nt - 1:
                        grp[gi][4]()
            return cc

        with jax.named_scope('attn_bwd'):
            lax.fori_loop(0, NG // BWD_UNROLL, attn_bwd, 0)

        def dw_proj(idx, lo=0, hi=D):
            v = awqkv_s[idx, lo:hi, :] + _dot(h1_s[s, lo:hi, :], dqkv_s[idx], _NT)
            awqkv_s[idx, lo:hi, :] = v
            dwqkv_v[idx, lo:hi, :] = v.astype(bf16)

        HL = L // 2

        def dh1_half(hf):
            acc1 = None
            for idx in range(3):
                t1 = _dot(dqkv_s[idx, :, hf * HL:(hf + 1) * HL], wqkv_ref[idx], _TN)
                acc1 = t1 if acc1 is None else acc1 + t1
            return acc1

        def ln1_bwd(hf, dh1):
            a0 = avec_s[0]
            a1 = avec_s[1]
            for rb in range(0, HL, RB):
                rows = pl.ds(pl.multiple_of(r0 + hf * HL + rb, RB), RB)
                xhat, rstd = _ln_stats(x_ref[rows, :].astype(f32))
                dh = dh1[rb:rb + RB]
                a1 = a1 + _colsum8(dh * xhat)
                a0 = a0 + _colsum8(dh)
                dx = (dx1_s[hf * HL + rb:hf * HL + rb + RB, :]
                      + _ln_bwd(dh * (1.0 + modv(1)), xhat, rstd))
                dx_v[rows, :] = dx.astype(bf16)
            avec_s[0] = a0
            avec_s[1] = a1

        dw_proj(0, 0, 128)
        dh1a = dh1_half(0)
        dh1b = dh1_half(1)
        ln1_bwd(0, dh1a)
        dw_proj(0, 128, D)
        ln1_bwd(1, dh1b)
        dwmod_cols(0, 2)
        dx_seg(s).start()

        @pl.when(last)
        def _():
            o_dwqkv[0].start()
            o_dwmod0.start()

        dw_proj(1)
        make_df(jnp.maximum(s - 1, 0), s > 0)

        @pl.when(last)
        def _():
            o_dwqkv[1].start()

        dw_proj(2)
        pl.when(last)(epilogue)
        return carry

    with jax.named_scope('phase2'):
        lax.fori_loop(0, NSEG, phase2, 0)


@jax.jit
def pallas_adaLN_cond__memory_aug_infini_attn__dense_activation_gelu__prompt_kernel(
    A_x: jax.Array,
    A_wq: jax.Array,
    A_wk: jax.Array,
    A_wv: jax.Array,
    A_wo: jax.Array,
    A_beta: jax.Array,
    B_x: jax.Array,
    B_w1: jax.Array,
    B_b1: jax.Array,
    B_w2: jax.Array,
    B_b2: jax.Array,
    c: jax.Array,
    w_mod: jax.Array,
    grad_out: jax.Array,
):
    sd = jax.ShapeDtypeStruct
    out_shape = (
        sd((S, D), bf16), sd((S, D), bf16),
        sd((D, D), bf16), sd((D, D), bf16), sd((D, D), bf16), sd((D, D), bf16),
        sd((F, D), bf16), sd((F, D), bf16), sd((D, 6 * D), bf16),
        sd((1, H), bf16), sd((F,), bf16), sd((D,), bf16), sd((1, D), bf16),
    )
    vm = pltpu.VMEM
    scratch = [
        vm((S, D), bf16), vm((S, D), bf16), vm((3, D, D), bf16), vm((D, D), bf16),
        vm((F, D), bf16), vm((F, D), bf16), vm((D, 6 * D), bf16),
        vm((3, D, D), bf16), vm((D, D), bf16),
        vm((F, D), bf16), vm((F, D), bf16), vm((D, 6 * D), bf16),
        vm((16, 6 * D), f32),
        vm((D, 128), f32),
        vm((NSEG, D, L), bf16),
        vm((NSEG, 3, D, L), bf16),
        vm((NSEG, NG, L, 128), bf16),
        vm((NSEG, NG, L, 128), bf16),
        vm((NSEG, NG, 96, GR), f32),
        vm((NG, 96, GR), f32),
        vm((NG, EROWS, 512), bf16),
        vm((EROWS, 512), f32), vm((EROWS, 512), f32),
        vm((NT, 16, 512), f32), vm((NT, 16, 512), f32),
        vm((NG, 32, L), f32),
        vm((NSEG, NG, 32, L), f32),
        vm((D, L), f32),
        vm((NSEG, D, L), f32),
        vm((D, L), bf16),
        vm((D, L), f32),
        vm((3, D, L), bf16),
        vm((L, D), f32),
        vm((3, D, D), f32), vm((D, D), f32), vm((F, D), f32), vm((F, D), f32),
        vm((7, 8, D), f32), vm((8, F), f32), vm((D, 128), f32),
        vm((6, L, 256), f32), vm((L, D), bf16), vm((D, 128), f32),
        vm((1, F), f32), vm((1, D), f32), vm((F - FT, 128), f32), vm((256, 128), f32),
        pltpu.SemaphoreType.DMA((12,)), pltpu.SemaphoreType.DMA((16,)),
    ]
    hbm = pl.BlockSpec(memory_space=pl.ANY)
    vmem = pl.BlockSpec(memory_space=pltpu.VMEM)
    outs = pl.pallas_call(
        _kernel,
        out_shape=out_shape,
        in_specs=[hbm] * 9 + [vmem] * 4,
        out_specs=tuple([hbm] * 9 + [vmem] * 4),
        scratch_shapes=scratch,
        compiler_params=pltpu.CompilerParams(vmem_limit_bytes=125 * 1024 * 1024),
    )(A_x.reshape(S, D), grad_out.reshape(S, D), A_wq, A_wk, A_wv, A_wo, B_w1.T, B_w2, w_mod,
      A_beta.reshape(1, H), B_b1, B_b2, c)
    (out, dx, dwq, dwk, dwv, dwo, dw1t, dw2, dwmod, dbeta, db1, db2, dc) = outs
    return (out.reshape(1, S, D), dx.reshape(1, S, D), dwq, dwk, dwv, dwo,
            dbeta.reshape(H), dw1t.T, db1, dw2, db2, dc, dwmod)
```

```python
import math

import jax
import jax.numpy as jnp
from jax import lax
import jax.experimental.pallas as pl
import jax.experimental.pallas.tpu as pltpu

S, D, H, DH, NSEG, L, F = 2048, 640, 32, 20, 4, 512, 1728
GR = 80
NG = D // GR
NT = L // 128
EROWS = 128 * NT * (NT + 1) // 2
EOFF = [128 * t * (t + 1) // 2 for t in range(NT)]
SCALE = DH ** (-0.5)
LOG2E = math.log2(math.e)
LN_EPS = 1e-5
DEN_EPS = 1e-6
NEG = -1e30
BWD_UNROLL = 4
BWD_LAG = 2
RB = 64
RB2 = 128
MEM_STEPS = (2, 5, 7, 9)
FT = 1536
FCHUNKS = [(0, 512), (512, 512), (1024, 512), (1536, 192)]

f32 = jnp.float32
bf16 = jnp.bfloat16

_NN = (((1,), (0,)), ((), ()))
_NT = (((1,), (1,)), ((), ()))
_TN = (((0,), (0,)), ((), ()))
_TT = (((0,), (1,)), ((), ()))


def _dot(a, b, dn):
    return lax.dot_general(a, b, dn, preferred_element_type=f32)


def _phi(t):
    return jnp.where(t > 0, t + 1.0, jnp.exp(t))


def _rows(shape):
    return lax.broadcasted_iota(jnp.int32, shape, 0)


def _cols(shape):
    return lax.broadcasted_iota(jnp.int32, shape, 1)


def _merge(parts):
    n = parts[0].shape[1]
    lo = _rows((8, n)) < 4
    a0, a1, a2, a3 = parts
    return jnp.concatenate([
        a0[0:16], jnp.where(lo, a0[16:24], a1[0:8]), a1[8:24],
        a2[0:16], jnp.where(lo, a2[16:24], a3[0:8]), a3[8:24]], axis=0)


def _expand(tiles):
    n = tiles[0].shape[1]
    lo = _rows((8, n)) < 4
    t0, t1, t2, t3 = tiles
    return jnp.concatenate([
        t0, t0, jnp.where(lo, t0, t1), t1, t1,
        t2, t2, jnp.where(lo, t2, t3), t3, t3], axis=0)


def _head_sums(a):
    n = a.shape[1]
    lo = _rows((8, n)) < 4
    z = jnp.zeros((8, n), a.dtype)
    p = [
        a[0:8] + a[8:16] + jnp.where(lo, a[16:24], z),
        jnp.where(lo, z, a[16:24]) + a[24:32] + a[32:40],
        a[40:48] + a[48:56] + jnp.where(lo, a[56:64], z),
        jnp.where(lo, z, a[56:64]) + a[64:72] + a[72:80],
    ]
    return [jnp.sum(t, axis=0, keepdims=True) for t in p]


def _rot64(a):
    return pltpu.roll(a, 64, 1)


def _pair_window(wa, wb):
    left = _cols((16, 128)) < 64
    ra = _rot64(wa)
    return jnp.concatenate([
        jnp.where(left, ra[0:16], 0.0), jnp.where(left, ra[16:32], wb[0:16]),
        jnp.where(left, 0.0, wb[16:32])], axis=0)


def _unpack_pairs(a):
    p0, p1 = a[:, 0:128], a[:, 128:256]
    return jnp.concatenate([_rot64(p0), p0, _rot64(p1), p1], axis=1)


def _lane_fold(a):
    return (a[:, 0:128] + a[:, 128:256]) + (a[:, 256:384] + a[:, 384:512])


def _ln_stats(x):
    mu = jnp.mean(x, axis=-1, keepdims=True)
    xc = x - mu
    var = jnp.mean(xc * xc, axis=-1, keepdims=True)
    rstd = lax.rsqrt(var + LN_EPS)
    return xc * rstd, rstd


def _ln_bwd(dxhat, xhat, rstd):
    m1 = jnp.mean(dxhat, axis=-1, keepdims=True)
    m2 = jnp.mean(dxhat * xhat, axis=-1, keepdims=True)
    return rstd * (dxhat - m1 - xhat * m2)


def _colsum8(a):
    r, n = a.shape
    return jnp.sum(a.reshape(r // 8, 8, n), axis=0)


def _kernel(x_hbm, g_hbm, wq_hbm, wk_hbm, wv_hbm, wo_hbm, w1_hbm, w2_hbm, wmod_hbm,
            beta_ref, b1_ref, b2_ref, c_ref,
            out_hbm, dx_hbm, dwq_hbm, dwk_hbm, dwv_hbm, dwo_hbm, dw1_hbm, dw2_hbm, dwmod_hbm,
            dbeta_ref, db1_ref, db2_ref, dc_ref,
            x_ref, g_ref, wqkv_ref, wo_ref, w1_ref, w2_ref, wmod_ref,
            dwqkv_v, dwo_v, dw1_v, dw2_v, dwmod_v,
            mod_s, gate_s, h1_s, qkv_s, ktm_s, vtm_s, mt_s, dmt_s, e_s, st0, st1, m0, m1,
            linv_s, dinv_s, adot_s, amem_s, ot_s, dot_s, dqkv_s, dx1_s,
            awqkv_s, awo_s, aw1_s, aw2_s, avec_s, ab1_s, adg_s, da_s, df_s, sccol_s, b1_s, b2_s, b1t_s, ab1t_s,
            isem, osem):
    out_v = g_ref
    dx_v = x_ref
    st_s = (st0, st1)
    m_s = (m0, m1)

    def cp(src, dst, sem):
        return pltpu.make_async_copy(src, dst, sem)

    in_wmod0 = cp(wmod_hbm.at[:, 0:2 * D], wmod_ref.at[:, 0:2 * D], isem.at[0])
    in_x0 = cp(x_hbm.at[0:L], x_ref.at[0:L], isem.at[1])
    in_wq = cp(wq_hbm, dwqkv_v.at[0], isem.at[2])
    in_wk = cp(wk_hbm, dwqkv_v.at[1], isem.at[3])
    in_wv = cp(wv_hbm, dwqkv_v.at[2], isem.at[4])
    in_x1 = cp(x_hbm.at[L:2 * L], x_ref.at[L:2 * L], isem.at[5])
    in_x2 = cp(x_hbm.at[2 * L:S], x_ref.at[2 * L:S], isem.at[11])
    in_wmod1 = cp(wmod_hbm.at[:, 2 * D:6 * D], wmod_ref.at[:, 2 * D:6 * D], isem.at[6])
    in_wo = cp(wo_hbm, wo_ref, isem.at[7])
    in_w1 = cp(w1_hbm, w1_ref, isem.at[8])
    in_w2 = cp(w2_hbm, w2_ref, isem.at[9])
    in_g = cp(g_hbm, g_ref, isem.at[10])

    def out_seg(s):
        r0 = pl.multiple_of(s * L, L)
        return cp(out_v.at[pl.ds(r0, L)], out_hbm.at[pl.ds(r0, L)], osem.at[s])

    def dx_seg(s):
        r0 = pl.multiple_of(s * L, L)
        return cp(dx_v.at[pl.ds(r0, L)], dx_hbm.at[pl.ds(r0, L)], osem.at[NSEG + s])

    o_dwqkv = [cp(dwqkv_v.at[i], dst, osem.at[8 + i])
               for i, dst in enumerate((dwq_hbm, dwk_hbm, dwv_hbm))]
    o_dwo = cp(dwo_v, dwo_hbm, osem.at[11])
    o_dw1 = cp(dw1_v, dw1_hbm, osem.at[12])
    o_dw2 = cp(dw2_v, dw2_hbm, osem.at[13])
    o_dwmod0 = cp(dwmod_v.at[:, 0:2 * D], dwmod_hbm.at[:, 0:2 * D], osem.at[14])
    o_dwmod1 = cp(dwmod_v.at[:, 2 * D:6 * D], dwmod_hbm.at[:, 2 * D:6 * D], osem.at[15])

    for d in (in_wmod0, in_x0, in_wk, in_wv):
        d.start()
    for r in (awo_s, avec_s, ab1_s, ab1t_s, adg_s, dmt_s, awqkv_s, aw1_s, aw2_s):
        r[...] = jnp.zeros(r.shape, r.dtype)
    mt_s[0] = jnp.zeros(mt_s.shape[1:], f32)
    c = c_ref[...].astype(f32)
    sig_c = jax.nn.sigmoid(c)
    silu_c = c * sig_c
    silu8 = jnp.broadcast_to(silu_c, (16, D)).astype(bf16)
    gate = jax.nn.sigmoid(beta_ref[...].astype(f32))
    hsel = (_rows((D, H)) // DH) == _cols((D, H))
    gcol = jnp.sum(jnp.where(hsel, gate, 0.0), axis=1, keepdims=True)
    gate_s[...] = jnp.broadcast_to(gcol, (D, 128))
    sccol_s[...] = jnp.broadcast_to(silu_c, (128, D)).T
    b1_s[...] = b1_ref[...].astype(f32).reshape(1, F)
    b2_s[...] = b2_ref[...].astype(f32).reshape(1, D)
    b1t_s[...] = jnp.concatenate(
        [jnp.broadcast_to(b1_s[:, FT:F], (128, F - FT)),
         jnp.zeros((128, 256 - (F - FT)), f32)], axis=1).T[0:F - FT]
    in_wmod0.wait()
    in_wq.start()
    in_x1.start()
    mod_s[:, 0:2 * D] = _dot(silu8, wmod_ref[:, 0:2 * D], _NN)
    in_x0.wait()

    def modv(i):
        return mod_s[0:1, i * D:(i + 1) * D]

    mr = _rows((96, GR))
    mc = _cols((96, GR)) // DH
    mem_mask = jnp.where(mr < GR, mr // DH, mr - GR) == mc

    def ln1_fwd(s):
        xhat, _ = _ln_stats(x_ref[s * L:(s + 1) * L, :].astype(f32))
        h1_s[s] = (xhat * (1.0 + modv(1)) + modv(0)).T.astype(bf16)

    def proj(idx, s):
        if s == 0:
            w = dwqkv_v[idx]
            wqkv_ref[idx] = w.T
            return _dot(w, h1_s[s], _TN)
        return _dot(wqkv_ref[idx], h1_s[s], _NN)

    def proj_k(s):
        kt = proj(1, s)
        qkv_s[s, 1] = kt.astype(bf16)
        for g in range(NG):
            ktm_s[s, g] = jnp.concatenate(
                [kt[g * GR:(g + 1) * GR] * (SCALE * LOG2E), jnp.zeros((48, L), f32)],
                axis=0).T.astype(bf16)

    def proj_v(s):
        vt = proj(2, s)
        qkv_s[s, 2] = vt.astype(bf16)
        for g in range(NG):
            vtm_s[s, g] = jnp.concatenate(
                [vt[g * GR:(g + 1) * GR], jnp.ones((16, L), f32), jnp.zeros((32, L), f32)],
                axis=0).T.astype(bf16)

    def proj_q(s):
        qt = proj(0, s)
        qkv_s[s, 0] = qt.astype(bf16)

    def mem_upd(s):
        ones = jnp.ones((16, L), bf16)
        for g in range(NG):
            rs = slice(g * GR, (g + 1) * GR)
            pk = _phi(qkv_s[s, 1, rs, :].astype(f32)).astype(bf16)
            vx = jnp.concatenate([qkv_s[s, 2, rs, :], ones], axis=0)
            upd = _dot(vx, pk, _NT)
            mt_s[s + 1, g] = mt_s[s, g] + jnp.where(mem_mask, upd, 0.0)

    def mem_read(s):
        if s == 0:
            dinv_s[0] = jnp.full(dinv_s.shape[1:], 1.0 / DEN_EPS, f32)
            amem_s[0] = jnp.zeros(amem_s.shape[1:], f32)
            return
        for g in range(NG):
            rs = slice(g * GR, (g + 1) * GR)
            pq = _phi(qkv_s[s, 0, rs, :].astype(f32)).astype(bf16)
            numx = _dot(mt_s[s, g].astype(bf16), pq, _NN)
            dinvs = [jnp.broadcast_to(1.0 / (numx[GR + j:GR + j + 1] + DEN_EPS), (8, L))
                     for j in range(4)]
            dinv_s[s, g] = jnp.concatenate(dinvs, axis=0)
            amem_s[s, rs, :] = numx[0:GR] * _expand(dinvs)

    ln1_fwd(0)
    mem_read(0)
    in_wk.wait()
    with jax.named_scope('phase1'):
        proj_k(0)
        in_wv.wait()
        in_x2.start()
        for s in range(NSEG):
            if s == 1:
                in_x2.wait()
                for d in (in_wmod1, in_g, in_w2, in_wo, in_w1):
                    d.start()
            if s > 0:
                proj_k(s)
                if s > 1:
                    mem_read(s - 1)
            if s + 1 < NSEG:
                proj_v(s)
                if s == 0:
                    in_wq.wait()
                    in_x1.wait()
                ln1_fwd(s + 1)
                proj_q(s)
                mem_upd(s)
            else:
                proj_q(s)
                proj_v(s)
                mem_read(s)

    in_wmod1.wait()
    mod_s[:, 2 * D:6 * D] = _dot(silu8, wmod_ref[:, 2 * D:6 * D], _NN)
    for d in (in_wo, in_w1, in_w2, in_g):
        d.wait()

    causal_t = _rows((64, 128)) <= _cols((64, 128))
    causal_t = jnp.concatenate([causal_t] * 4, axis=1)
    causal_b = _rows((64, 128)) <= (_cols((64, 128)) & 63)
    causal_b = jnp.concatenate([causal_b] * 2, axis=1)
    upper8 = jnp.concatenate([_cols((8, 128)) >= 64] * 4, axis=1)
    upper64 = jnp.concatenate([upper8] * 8, axis=0)
    wrow = _rows((32, L))
    r16 = _rows((16, L))
    inh = [(wrow >= 4 * j) & (wrow < 4 * j + DH) for j in range(4)]
    los = (0, 0, 8, 8)

    def dwmod_cols(lo, hi):
        sc_col = jnp.concatenate([sccol_s[...]] * (D // 128), axis=1)
        for i in range(lo, hi):
            dm = jnp.sum(avec_s[i], axis=0, keepdims=True)
            dwmod_v[:, i * D:(i + 1) * D] = (sc_col * dm).astype(bf16)

    def make_df(s, valid):
        gsum = None
        for rb in range(0, L, 64):
            gout = g_ref[pl.ds(pl.multiple_of(s * L + rb, 64), 64), :].astype(f32)
            df_s[rb:rb + 64, :] = (gout * (0.5 * modv(5))).astype(bf16)
            gsum = _colsum8(gout) if gsum is None else gsum + _colsum8(gout)
        avec_s[6] += jnp.where(valid, gsum, 0.0)

    make_df(NSEG - 1, True)

    def epilogue():
        o_dwqkv[2].start()
        rr = _rows((16, D))
        dsc = jnp.zeros((16, D), f32)
        for i in range(6):
            dm = jnp.sum(avec_s[i], axis=0, keepdims=True)
            hi_p = dm.astype(bf16).astype(f32)
            lhs = jnp.where(rr == 0, hi_p, jnp.where(rr == 1, dm - hi_p, 0.0)).astype(bf16)
            dsc = dsc + _dot(lhs, wmod_ref[:, i * D:(i + 1) * D], _NT)
        ab1_s[:, FT:F] = _colsum8(ab1t_s[...].T)[:, 0:F - FT]
        db1_ref[...] = jnp.sum(ab1_s[...], axis=0).astype(bf16)
        db2_ref[...] = jnp.sum(avec_s[6] * modv(5), axis=0).astype(bf16)
        dgc = jnp.sum(adg_s[...], axis=1, keepdims=True)
        dg = jnp.sum(jnp.where(hsel, dgc, 0.0), axis=0, keepdims=True)
        dbeta_ref[...] = (dg * gate * (1.0 - gate)).astype(bf16)
        dsilu = sig_c * (1.0 + c * (1.0 - sig_c))
        dc_ref[...] = ((dsc[0:1] + dsc[1:2]) * dsilu).astype(bf16)
        for s in range(NSEG):
            out_seg(s).wait()
            dx_seg(s).wait()
        for d in o_dwqkv + [o_dwo, o_dw1, o_dw2, o_dwmod0, o_dwmod1]:
            d.wait()

    def phase2(i, carry):
        s = NSEG - 1 - i
        r0 = pl.multiple_of(s * L, L)
        last = i == NSEG - 1

        def a_prep(g):
            g0 = pl.multiple_of(g * GR, 16)
            qs = qkv_s[s, 0, pl.ds(g0, GR), :]
            rhs, qws = [], []
            for j in range(4):
                qw = jnp.where(inh[j], qs[16 * j:16 * j + 32].astype(f32), 0.0)
                qws.append(qw)
                pieces = []
                if j > 0:
                    pieces.append(jnp.zeros((16 * j, L), bf16))
                pieces.append(qw.astype(bf16))
                pieces.append(jnp.zeros((96 - 16 * j, L), bf16))
                rhs.append(jnp.concatenate(pieces, axis=0))
            return rhs, qws

        def a_tile(g, prep, slot, t):
            rhs, qws = prep
            n = 128 * (t + 1)
            cs = slice(128 * t, n)
            r = jnp.concatenate([rhs[j][:, cs] for j in range(4)], axis=1)
            st = _dot(ktm_s[s, g, 0:n - 64, :], r, _NN)
            w0 = _pair_window(qws[0][:, cs], qws[1][:, cs]).astype(bf16)
            w1 = _pair_window(qws[2][:, cs], qws[3][:, cs]).astype(bf16)
            rp = jnp.concatenate([
                jnp.concatenate([w0, jnp.zeros((80, 128), bf16)], axis=0),
                jnp.concatenate([jnp.zeros((32, 128), bf16), w1, jnp.zeros((48, 128), bf16)],
                                axis=0)], axis=1)
            bot = jnp.where(causal_b, _dot(ktm_s[s, g, n - 64:n, :], rp, _NN), NEG)
            diag = jnp.where(causal_t, st[n - 128:n - 64], NEG)
            st = jnp.concatenate([st[0:n - 128], diag], axis=0) if t > 0 else diag
            st_s[slot][EOFF[t]:EOFF[t] + n - 64, :] = st
            st_s[slot][EOFF[t] + n - 64:EOFF[t] + n, 0:256] = bot
            mb = jnp.broadcast_to(jnp.max(bot, axis=0, keepdims=True), (8, 256))
            mt = jnp.broadcast_to(jnp.max(st, axis=0, keepdims=True), (8, 512))
            mx = jnp.where(upper8, jnp.maximum(mt, _unpack_pairs(mb)), mt)
            m_s[slot][t, 0:8, :] = mx
            m_s[slot][t, 8:16, 0:256] = jnp.concatenate(
                [jnp.where(upper8[:, 0:128], mx[:, 128 * (j + 1):128 * (j + 2)],
                           _rot64(mx[:, 128 * j:128 * (j + 1)])) for j in (0, 2)], axis=1)

        def b_prep(g):
            g0 = pl.multiple_of(g * GR, 16)
            vt = qkv_s[s, 2, pl.ds(g0, GR), :]
            return [jnp.where(inh[j], vt[16 * j:16 * j + 32].astype(f32), 1.0).astype(bf16)
                    for j in range(4)]

        def b_tile(g, vws, slot, t):
            n = 128 * (t + 1)
            e32 = jnp.exp2(st_s[slot][EOFF[t]:EOFF[t] + n - 64, :] - m_s[slot][t, 0:1, :])
            eb = jnp.exp2(st_s[slot][EOFF[t] + n - 64:EOFF[t] + n, 0:256]
                          - m_s[slot][t, 8:9, 0:256])
            e32 = jnp.concatenate([e32, jnp.where(upper64, _unpack_pairs(eb), 0.0)], axis=0)
            e_s[g, EOFF[t]:EOFF[t] + n, :] = e32.astype(bf16)
            return [_dot(vws[j][:, 0:n], e32[:, 128 * j:128 * (j + 1)].astype(bf16), _NN)
                    for j in range(4)]

        def b_fin(g, pv):
            g0 = pl.multiple_of(g * GR, 16)
            parts, linvs = [], []
            for j in range(4):
                ow = jnp.concatenate([pv[t][j] for t in range(NT)], axis=1)
                linv = 1.0 / (ow[24:32] if j < 2 else ow[0:8])
                linvs.append(linv)
                parts.append(ow[los[j]:los[j] + 24] * jnp.concatenate([linv] * 3, axis=0))
            adot = _merge(parts)
            linv_s[g] = jnp.concatenate(linvs, axis=0)
            adot_s[pl.ds(g0, GR), :] = adot
            gt = jnp.concatenate([gate_s[pl.ds(g0, GR), :]] * NT, axis=1)
            amem = amem_s[s, pl.ds(g0, GR), :]
            ot_s[pl.ds(g0, GR), :] = (gt * amem + (1.0 - gt) * adot).astype(bf16)

        def da_slice(k, lo, hi):
            c0 = pl.multiple_of(k * 256, 256)
            da_s[k, lo:hi, :] = _dot(df_s[lo:hi, :], w2_ref[pl.ds(c0, 256), :], _NT)

        def ab(g, slot):
            rhs = a_prep(g + 1)
            vws = b_prep(g)
            pv = []
            for t in range(NT):
                a_tile(g + 1, rhs, 1 - slot, t)
                if not (isinstance(g, int) and g == NG - 2):
                    da_slice(g, 128 * t, 128 * (t + 1))
                pv.append(b_tile(g, vws, slot, t))
            b_fin(g, pv)

        def fwd_pair(p, cc):
            ab(2 * p, 0)
            ab(2 * p + 1, 1)
            return cc

        with jax.named_scope('attn_fwd'):
            rhs0 = a_prep(0)
            for t in range(NT):
                a_tile(0, rhs0, 0, NT - 1 - t)
            lax.fori_loop(0, NG // 2 - 1, fwd_pair, 0)
            ab(NG - 2, 0)
            vws = b_prep(NG - 1)
            pv = [b_tile(NG - 1, vws, 1, 0)]
            att = _dot(ot_s[0:256, :], wo_ref[0:256, :], _TN)
            pv += [b_tile(NG - 1, vws, 1, t) for t in range(1, 3)]
            att = att + _dot(ot_s[256:512, :], wo_ref[256:512, :], _TN)
            pv.append(b_tile(NG - 1, vws, 1, 3))
            b_fin(NG - 1, pv)

        att = att + _dot(ot_s[512:D, :], wo_ref[512:D, :], _TN)
        df = df_s[...]
        da_t = _dot(w2_ref[FT:F, :], df, _NT)
        x1s, xhs, rss, h2s = [], [], [], []
        for rb in range(0, L, 64):
            rows = pl.ds(pl.multiple_of(r0 + rb, 64), 64)
            x1b = x_ref[rows, :].astype(f32) + modv(2) * att[rb:rb + 64]
            xh, rsd = _ln_stats(x1b)
            x1s.append(x1b)
            xhs.append(xh)
            rss.append(rsd)
            h2s.append((xh * (1.0 + modv(4)) + modv(3)).astype(bf16))
        x1 = jnp.concatenate(x1s, axis=0)
        xhat2 = jnp.concatenate(xhs, axis=0)
        rstd2 = jnp.concatenate(rss, axis=0)
        h2 = jnp.concatenate(h2s, axis=0)
        k0 = math.sqrt(2.0 / math.pi)
        k1 = 0.044715

        def gelu2(u, da):
            u2 = u * u
            th = jnp.tanh(u * (k0 + (k0 * k1) * u2))
            t1 = 1.0 + th
            a2 = u * t1
            gp = t1 + a2 * (1.0 - th) * (k0 + (3.0 * k0 * k1) * u2)
            return a2.astype(bf16), da * gp

        def ffn_up(c0, cw):
            cs = slice(c0, c0 + cw)
            if c0 == FT:
                u = (_dot(w1_ref[cs, :], h2, _NT)
                     + jnp.concatenate([b1t_s[...]] * NT, axis=1))
                a, duf = gelu2(u, da_t)
                ab1t_s[0:cw, :] += _lane_fold(duf)
                return a, duf.astype(bf16)
            u = _dot(h2, w1_ref[cs, :], _NT) + b1_s[:, cs]
            da = jnp.concatenate([da_s[k] for k in range(c0 // 256, (c0 + cw) // 256)], axis=1)
            a, duf = gelu2(u, da)
            ab1_s[:, cs] += _colsum8(duf)
            return a, duf.astype(bf16)

        def ffn_dw(c0, cw, a, du):
            cs = slice(c0, c0 + cw)
            dn = _NN if c0 == FT else _TN
            v2 = aw2_s[cs, :] + _dot(a, df, dn)
            aw2_s[cs, :] = v2
            dw2_v[cs, :] = v2.astype(bf16)
            v1 = aw1_s[cs, :] + _dot(du, h2, dn)
            aw1_s[cs, :] = v1
            dw1_v[cs, :] = v1.astype(bf16)

        facc = None
        dh2 = None
        ups = [ffn_up(*FCHUNKS[0])]
        for ci, (c0, cw) in enumerate(FCHUNKS):
            cs = slice(c0, c0 + cw)
            if ci + 1 < len(FCHUNKS):
                ups.append(ffn_up(*FCHUNKS[ci + 1]))
            a, du = ups[ci]
            dn = _TN if c0 == FT else _NN
            t1 = _dot(du, w1_ref[cs, :], dn)
            dh2 = t1 if dh2 is None else dh2 + t1
            t2 = _dot(a, w2_ref[cs, :], dn)
            facc = t2 if facc is None else facc + t2
            if ci < len(FCHUNKS) - 2:
                ffn_dw(c0, cw, a, du)
        for ci in range(len(FCHUNKS) - 2, len(FCHUNKS)):
            ffn_dw(*FCHUNKS[ci], *ups[ci])
        av = [avec_s[k] for k in range(2, 6)]
        b2 = b2_s[...]
        datts = []
        for rb in range(0, L, RB2):
            rs = slice(rb, rb + RB2)
            rows = pl.ds(pl.multiple_of(r0 + rb, RB2), RB2)
            gout = g_ref[rows, :].astype(f32)
            ff = 0.5 * facc[rs] + b2
            dh = dh2[rs]
            av[3] = av[3] + _colsum8(gout * ff)
            av[2] = av[2] + _colsum8(dh * xhat2[rs])
            av[1] = av[1] + _colsum8(dh)
            dx1 = gout + _ln_bwd(dh * (1.0 + modv(4)), xhat2[rs], rstd2[rs])
            dx1_s[rs, :] = dx1
            out_v[rows, :] = (x1[rs] + modv(5) * ff).astype(bf16)
            av[0] = av[0] + _colsum8(dx1 * att[rs])
            datts.append((dx1 * modv(2)).astype(bf16))
        for k in range(4):
            avec_s[2 + k] = av[k]
        datt = jnp.concatenate(datts, axis=0)
        dot_s[...] = _dot(wo_ref[...], datt, _NT)
        vo = awo_s[...] + _dot(ot_s[...], datt, _NN)
        awo_s[...] = vo
        dwo_v[...] = vo.astype(bf16)
        out_seg(s).start()


        def bwd_group(g, mode):
            g0 = pl.multiple_of(g * GR, 16)
            do = dot_s[pl.ds(g0, GR), :]
            adot = adot_s[pl.ds(g0, GR), :]
            gt = jnp.concatenate([gate_s[pl.ds(g0, GR), :]] * NT, axis=1)
            linv = linv_s[g]
            qt = qkv_s[s, 0, pl.ds(g0, GR), :]
            kt = qkv_s[s, 1, pl.ds(g0, GR), :]
            dop = ((1.0 - gt) * do
                   * _expand([linv[8 * j:8 * j + 8] for j in range(4)])).astype(bf16)
            dopf = dop.astype(f32)
            deltas = _head_sums(dopf * adot)
            rhs, dws, drows = [], [], []
            for j in range(4):
                dw = jnp.where(inh[j], dopf[16 * j:16 * j + 32], 0.0)
                nd = -deltas[j]
                nd_hi = nd.astype(bf16).astype(f32)
                drow = jnp.where(r16 == 0, nd_hi, jnp.where(r16 == 1, nd - nd_hi, 0.0))
                dws.append(dw)
                drows.append(drow)
                pieces = []
                if j > 0:
                    pieces.append(jnp.zeros((16 * j, L), bf16))
                pieces.append(dw.astype(bf16))
                if j < 3:
                    pieces.append(jnp.zeros((48 - 16 * j, L), bf16))
                pieces.append(drow.astype(bf16))
                pieces.append(jnp.zeros((32, L), bf16))
                rhs.append(jnp.concatenate(pieces, axis=0))
            rt = [jnp.concatenate([rhs[j][:, 128 * t:128 * (t + 1)] for j in range(4)], axis=1)
                  for t in range(NT)]

            def packed_rhs(t):
                cs = slice(128 * t, 128 * (t + 1))
                cols = []
                for j in (0, 2):
                    win = _pair_window(dws[j][:, cs], dws[j + 1][:, cs])
                    dr = jnp.where(_cols((16, 128)) < 64, _rot64(drows[j][:, cs]),
                                   drows[j + 1][:, cs])
                    pieces = [win.astype(bf16), jnp.zeros((32, 128), bf16)]
                    if j:
                        pieces = pieces[::-1]
                    cols.append(jnp.concatenate(
                        pieces + [dr.astype(bf16), jnp.zeros((32, 128), bf16)], axis=0))
                return jnp.concatenate(cols, axis=1)

            kw = [kt[16 * j:16 * j + 32] for j in range(4)]
            qw = [qt[16 * j:16 * j + 32] for j in range(4)]
            dow = [dop[16 * j:16 * j + 32] for j in range(4)]
            dq_t = [[None] * NT for _ in range(4)]
            dk_t = [[None] * NT for _ in range(4)]
            dv_t = [[None] * NT for _ in range(4)]
            mem_out = {}

            def acc(lst, k, val):
                lst[k] = val if lst[k] is None else lst[k] + val

            def f_dp(t, u):
                e0 = EOFF[t] + 128 * u
                if u < t:
                    dp = _dot(vtm_s[s, g, 128 * u:128 * (u + 1), :], rt[t], _NN)
                else:
                    top = _dot(vtm_s[s, g, 128 * u:128 * u + 64, :], rt[t], _NN)
                    bot = _dot(vtm_s[s, g, 128 * u + 64:128 * (u + 1), :], packed_rhs(t), _NN)
                    dp = jnp.concatenate([top, _unpack_pairs(bot)], axis=0)
                ds = e_s[g, e0:e0 + 128, :].astype(f32) * dp
                return [ds[:, 128 * j:128 * (j + 1)].astype(bf16) for j in range(4)]

            def f_dv(t, u):
                e0 = EOFF[t] + 128 * u
                for j in range(4):
                    e = e_s[g, e0:e0 + 128, 128 * j:128 * (j + 1)]
                    acc(dv_t[j], u, _dot(dow[j][:, 128 * t:128 * (t + 1)], e, _NT))

            def f_dqk(t, u, ds):
                for j in range(4):
                    acc(dk_t[j], u, _dot(qw[j][:, 128 * t:128 * (t + 1)], ds[j], _NT))
                for j in range(4):
                    acc(dq_t[j], t, _dot(kw[j][:, 128 * u:128 * (u + 1)], ds[j], _NN))

            def f_mem(step):
                m = mem_out
                if step == 0 and mode != 0:
                    m['dmt'] = dmt_s[g]
                    m['dmtb'] = m['dmt'].astype(bf16)
                    vt = qkv_s[s, 2, pl.ds(g0, GR), :]
                    vx = jnp.concatenate([vt, jnp.ones((16, L), bf16)], axis=0)
                    kf = kt.astype(f32)
                    m['pkf'] = _phi(kf)
                    m['dk'] = (_dot(m['dmtb'], vx, _TN)
                               * jnp.where(kf > 0, 1.0, m['pkf']))
                elif step == 1:
                    if mode != 0:
                        m['dv'] = _dot(m['dmtb'][0:GR], m['pkf'].astype(bf16), _NN)
                    amem = amem_s[s, pl.ds(g0, GR), :]
                    adg_s[pl.ds(g0, GR), :] += _lane_fold(do * (amem - adot))
                    if mode != 2:
                        dinv = dinv_s[s, g]
                        dnum = gt * do * _expand([dinv[8 * j:8 * j + 8] for j in range(4)])
                        dds = _head_sums(dnum * amem)
                        dden = jnp.zeros((16, L), f32)
                        for j in range(4):
                            dden = jnp.where(r16 == j, -dds[j], dden)
                        m['dnx'] = jnp.concatenate([dnum, dden], axis=0).astype(bf16)
                elif step == 2 and mode != 2:
                    qf = qt.astype(f32)
                    m['pqf'] = _phi(qf)
                    m['dq'] = (_dot(mt_s[s, g].astype(bf16), m['dnx'], _TN)
                               * jnp.where(qf > 0, 1.0, m['pqf']))
                elif step == 3 and mode != 2:
                    upd = jnp.where(mem_mask, _dot(m['dnx'], m['pqf'].astype(bf16), _NT), 0.0)
                    dmt_s[g] = upd if mode == 0 else m['dmt'] + upd

            def f_fin():
                def mg(lst):
                    return _merge([jnp.concatenate(lst[j], axis=1)[los[j]:los[j] + 24]
                                   for j in range(4)])

                vals = (mg(dq_t) * SCALE, mg(dk_t) * SCALE, mg(dv_t))
                for idx, key in enumerate(('dq', 'dk', 'dv')):
                    v = vals[idx] + mem_out[key] if key in mem_out else vals[idx]
                    dqkv_s[idx, pl.ds(g0, GR), :] = v.astype(bf16)

            return f_dp, f_dv, f_dqk, f_mem, f_fin

        def attn_bwd(mode, p, cc):
            tl = [(t, u) for t in range(NT) for u in range(t + 1)]
            nt = len(tl)
            grp = [bwd_group(BWD_UNROLL * p, mode)]
            dss = {}
            for k in range(BWD_UNROLL * nt + BWD_LAG):
                if k < BWD_UNROLL * nt:
                    gi, ti = divmod(k, nt)
                    if ti == 6 and gi + 1 < BWD_UNROLL:
                        grp.append(bwd_group(BWD_UNROLL * p + gi + 1, mode))
                    dss[k] = grp[gi][0](*tl[ti])
                    grp[gi][1](*tl[ti])
                    if ti in MEM_STEPS:
                        grp[gi][3](MEM_STEPS.index(ti))
                    if mode == 2 and ti in (7, 9):
                        ci = 2 + 2 * p + gi // 2
                        rs = slice((2 * (gi % 2) + (ti == 9)) * (D // 4),
                                   (2 * (gi % 2) + (ti == 9) + 1) * (D // 4))
                        dm = jnp.sum(avec_s[ci], axis=0, keepdims=True)
                        sc_col = jnp.concatenate([sccol_s[rs, :]] * (D // 128), axis=1)
                        dwmod_v[rs, pl.ds(pl.multiple_of(ci * D, 128), D)] = (
                            sc_col * dm).astype(bf16)
                if k >= BWD_LAG:
                    gi, ti = divmod(k - BWD_LAG, nt)
                    grp[gi][2](*tl[ti], dss.pop(k - BWD_LAG))
                    if ti == nt - 1:
                        grp[gi][4]()
            return cc

        with jax.named_scope('attn_bwd'):
            for mode in (1, 2):
                @pl.when(last == (mode == 2))
                def _(mode=mode):
                    if mode == 2:
                        o_dw1.start()
                        o_dw2.start()
                        o_dwo.start()
                    lax.fori_loop(0, NG // BWD_UNROLL,
                                  lambda p, cc: attn_bwd(mode, p, cc), 0)
                    if mode == 2:
                        o_dwmod1.start()

        def dw_proj(idx, lo=0, hi=D):
            v = awqkv_s[idx, lo:hi, :] + _dot(h1_s[s, lo:hi, :], dqkv_s[idx], _NT)
            awqkv_s[idx, lo:hi, :] = v
            dwqkv_v[idx, lo:hi, :] = v.astype(bf16)

        HL = L // 2

        def dh1_half(hf):
            acc1 = None
            for idx in range(3):
                t1 = _dot(dqkv_s[idx, :, hf * HL:(hf + 1) * HL], wqkv_ref[idx], _TN)
                acc1 = t1 if acc1 is None else acc1 + t1
            return acc1

        def ln1_bwd(hf, dh1):
            a0 = avec_s[0]
            a1 = avec_s[1]
            for rb in range(0, HL, RB):
                rows = pl.ds(pl.multiple_of(r0 + hf * HL + rb, RB), RB)
                xhat, rstd = _ln_stats(x_ref[rows, :].astype(f32))
                dh = dh1[rb:rb + RB]
                a1 = a1 + _colsum8(dh * xhat)
                a0 = a0 + _colsum8(dh)
                dx = (dx1_s[hf * HL + rb:hf * HL + rb + RB, :]
                      + _ln_bwd(dh * (1.0 + modv(1)), xhat, rstd))
                dx_v[rows, :] = dx.astype(bf16)
            avec_s[0] = a0
            avec_s[1] = a1

        dw_proj(0, 0, 128)
        dh1a = dh1_half(0)
        dh1b = dh1_half(1)
        ln1_bwd(0, dh1a)
        dw_proj(0, 128, D)
        ln1_bwd(1, dh1b)
        dwmod_cols(0, 2)
        dx_seg(s).start()

        @pl.when(last)
        def _():
            o_dwqkv[0].start()
            o_dwmod0.start()

        dw_proj(1)
        make_df(jnp.maximum(s - 1, 0), s > 0)

        @pl.when(last)
        def _():
            o_dwqkv[1].start()

        dw_proj(2)
        pl.when(last)(epilogue)
        return carry

    with jax.named_scope('phase2'):
        lax.fori_loop(0, NSEG, phase2, 0)


@jax.jit
def pallas_adaLN_cond__memory_aug_infini_attn__dense_activation_gelu__prompt_kernel(
    A_x: jax.Array,
    A_wq: jax.Array,
    A_wk: jax.Array,
    A_wv: jax.Array,
    A_wo: jax.Array,
    A_beta: jax.Array,
    B_x: jax.Array,
    B_w1: jax.Array,
    B_b1: jax.Array,
    B_w2: jax.Array,
    B_b2: jax.Array,
    c: jax.Array,
    w_mod: jax.Array,
    grad_out: jax.Array,
):
    sd = jax.ShapeDtypeStruct
    out_shape = (
        sd((S, D), bf16), sd((S, D), bf16),
        sd((D, D), bf16), sd((D, D), bf16), sd((D, D), bf16), sd((D, D), bf16),
        sd((F, D), bf16), sd((F, D), bf16), sd((D, 6 * D), bf16),
        sd((1, H), bf16), sd((F,), bf16), sd((D,), bf16), sd((1, D), bf16),
    )
    vm = pltpu.VMEM
    scratch = [
        vm((S, D), bf16), vm((S, D), bf16), vm((3, D, D), bf16), vm((D, D), bf16),
        vm((F, D), bf16), vm((F, D), bf16), vm((D, 6 * D), bf16),
        vm((3, D, D), bf16), vm((D, D), bf16),
        vm((F, D), bf16), vm((F, D), bf16), vm((D, 6 * D), bf16),
        vm((16, 6 * D), f32),
        vm((D, 128), f32),
        vm((NSEG, D, L), bf16),
        vm((NSEG, 3, D, L), bf16),
        vm((NSEG, NG, L, 128), bf16),
        vm((NSEG, NG, L, 128), bf16),
        vm((NSEG, NG, 96, GR), f32),
        vm((NG, 96, GR), f32),
        vm((NG, EROWS, 512), bf16),
        vm((EROWS, 512), f32), vm((EROWS, 512), f32),
        vm((NT, 16, 512), f32), vm((NT, 16, 512), f32),
        vm((NG, 32, L), f32),
        vm((NSEG, NG, 32, L), f32),
        vm((D, L), f32),
        vm((NSEG, D, L), f32),
        vm((D, L), bf16),
        vm((D, L), f32),
        vm((3, D, L), bf16),
        vm((L, D), f32),
        vm((3, D, D), f32), vm((D, D), f32), vm((F, D), f32), vm((F, D), f32),
        vm((7, 8, D), f32), vm((8, F), f32), vm((D, 128), f32),
        vm((6, L, 256), f32), vm((L, D), bf16), vm((D, 128), f32),
        vm((1, F), f32), vm((1, D), f32), vm((F - FT, 128), f32), vm((256, 128), f32),
        pltpu.SemaphoreType.DMA((12,)), pltpu.SemaphoreType.DMA((16,)),
    ]
    hbm = pl.BlockSpec(memory_space=pl.ANY)
    vmem = pl.BlockSpec(memory_space=pltpu.VMEM)
    outs = pl.pallas_call(
        _kernel,
        out_shape=out_shape,
        in_specs=[hbm] * 9 + [vmem] * 4,
        out_specs=tuple([hbm] * 9 + [vmem] * 4),
        scratch_shapes=scratch,
        compiler_params=pltpu.CompilerParams(vmem_limit_bytes=125 * 1024 * 1024),
    )(A_x.reshape(S, D), grad_out.reshape(S, D), A_wq, A_wk, A_wv, A_wo, B_w1.T, B_w2, w_mod,
      A_beta.reshape(1, H), B_b1, B_b2, c)
    (out, dx, dwq, dwk, dwv, dwo, dw1t, dw2, dwmod, dbeta, db1, db2, dc) = outs
    return (out.reshape(1, S, D), dx.reshape(1, S, D), dwq, dwk, dwv, dwo,
            dbeta.reshape(H), dw1t.T, db1, dw2, db2, dc, dwmod)
```
